```python
import jax
import jax.numpy as jnp

def _softmax(x, axis=-1):
    return jax.nn.softmax(x, axis=axis)

def _gelu(x):
    return jax.nn.gelu(x, approximate=True)

def _silu(x):
    return jax.nn.silu(x)

def _sigmoid(x):
    return jax.nn.sigmoid(x)

def _layernorm(x, axis=-1, eps=1e-05):
    m = jnp.mean(x, axis=axis, keepdims=True)
    v = jnp.var(x, axis=axis, keepdims=True)
    return (x - m) / jnp.sqrt(v + eps)

def _scatter_add(tgt, idx, src, axis=0):
    return tgt.at[idx].add(src)

def _segment_sum(src, seg, n):
    return jax.ops.segment_sum(src, seg, n)

class _Rng:

    def __init__(self, key):
        self._k = key

    def _next(self):
        self._k, sub = jax.random.split(self._k)
        return sub

    def normal(self, shape):
        return jax.random.normal(self._next(), shape, dtype=jnp.bfloat16)

    def randint(self, lo, hi, shape):
        return jax.random.randint(self._next(), shape, lo, hi, dtype=jnp.int32)

    def uniform(self, shape, lo=0.0, hi=1.0):
        return jax.random.uniform(self._next(), shape, jnp.bfloat16, lo, hi)

    def permutation(self, n):
        return jax.random.permutation(self._next(), n)
kernel_name = 'interleave_layers__memory_aug_recurrent_mem_tr__linear_kernel_hedgehog__prompt'

def setup_inputs():
    _rng = _Rng(jax.random.key(int.from_bytes(__import__("os").urandom(4), "little")))
    _w = lambda a: (lambda t: t.astype(jnp.bfloat16) if jnp.issubdtype(t.dtype, jnp.floating) else t)(jnp.asarray(a))

    def _A_setup():
        B, S, Dm = (1, 2048, 640)
        H, Dh = (32, 192)
        M, seg = (8, 32)
        seg = min(seg, S)
        S = S // seg * seg
        return {'x': _w((lambda *s: _rng.normal(s) * 0.05)(B, S, Dm)), 'mem0': _w((lambda *s: _rng.normal(s) * 0.05)(B, M, Dm)), 'Wq': _w((lambda *s: _rng.normal(s) * 0.05)(Dm, H, Dh) * Dm ** (-0.5)), 'Wk': _w((lambda *s: _rng.normal(s) * 0.05)(Dm, H, Dh) * Dm ** (-0.5)), 'Wv': _w((lambda *s: _rng.normal(s) * 0.05)(Dm, H, Dh) * Dm ** (-0.5)), 'Wo': _w((lambda *s: _rng.normal(s) * 0.05)(H, Dh, Dm) * (H * Dh) ** (-0.5)), 'seg_len': seg}
    _A_in = _A_setup()

    def _B_setup():
        B, S, D, H = (1, 2048, 640, 32)
        Dh = D // H
        return {'x': _w((lambda *s: _rng.normal(s) * 0.05)(B, S, D)), 'wqkv': _w((lambda *s: _rng.normal(s) * 0.05)(D, 3 * D)), 'w_phi': _w((lambda *s: _rng.normal(s) * 0.05)(H, Dh, Dh) * Dh ** (-0.5)), 'wo': _w((lambda *s: _rng.normal(s) * 0.05)(D, D))}
    _B_in = _B_setup()
    return {'A_x': _A_in['x'], 'A_mem0': _A_in['mem0'], 'A_Wq': _A_in['Wq'], 'A_Wk': _A_in['Wk'], 'A_Wv': _A_in['Wv'], 'A_Wo': _A_in['Wo'], 'A_seg_len': _A_in['seg_len'], 'B_x': _B_in['x'], 'B_wqkv': _B_in['wqkv'], 'B_w_phi': _B_in['w_phi'], 'B_wo': _B_in['wo']}

def reference(A_x, A_mem0, A_Wq, A_Wk, A_Wv, A_Wo, A_seg_len, B_x, B_wqkv, B_w_phi, B_wo):

    def _A_ref(x, mem0, Wq, Wk, Wv, Wo, seg_len):
        B, S, Dm = x.shape
        H, Dh = (Wq.shape[1], Wq.shape[2])
        M = mem0.shape[1]
        scale = Dh ** (-0.5)
        n_seg = S // seg_len
        L = M + seg_len
        idx = jnp.arange(L)
        mask = (idx[:, None] < M) | (idx[:, None] >= idx[None, :])
        mem = mem0
        outs = []
        for s in range(n_seg):
            xs = x[:, s * seg_len:(s + 1) * seg_len, :].copy()
            h = jnp.concatenate([mem, xs], axis=1)
            q = jnp.einsum('btd,dhe->bhte', h, Wq)
            k = jnp.einsum('btd,dhe->bhte', h, Wk)
            v = jnp.einsum('btd,dhe->bhte', h, Wv)
            scores = jnp.einsum('bhqe,bhke->bhqk', q, k) * scale
            scores = jnp.where(mask[None, None], scores, -1000000000.0)
            p = _softmax(scores, axis=-1)
            o = jnp.einsum('bhqk,bhke->bhqe', p, v)
            o = jnp.einsum('bhte,hed->btd', o, Wo)
            mem = o[:, :M, :].copy()
            outs.append(o[:, M:, :])
        return jnp.concatenate(outs, axis=1)

    def _B_ref(x, wqkv, w_phi, wo):
        B, S, D = x.shape
        H = 32
        Dh = D // H
        qkv = (lambda x, *d: x.transpose(*d))((x @ wqkv).reshape(B, S, 3, H, Dh), 2, 0, 3, 1, 4)
        q, k, v = (qkv[0], qkv[1], qkv[2])
        pq = jnp.einsum('bhsd,hdf->bhsf', q, w_phi)
        pk = jnp.einsum('bhsd,hdf->bhsf', k, w_phi)
        phi_q = jnp.concatenate([_softmax(pq, axis=-1), _softmax(-pq, axis=-1)], axis=-1)
        phi_k = jnp.concatenate([_softmax(pk, axis=-1), _softmax(-pk, axis=-1)], axis=-1)
        kv = jnp.einsum('bhsf,bhsd->bhfd', phi_k, v)
        z = jnp.einsum('bhsf->bhf', phi_k)
        num = jnp.einsum('bhqf,bhfd->bhqd', phi_q, kv)
        den = jnp.einsum('bhqf,bhf->bhq', phi_q, z)[..., None] + 1e-06
        o = num / den
        return (lambda x, *d: x.transpose(*d))(o, 0, 2, 1, 3).reshape(B, S, D) @ wo
    x = A_x
    x = x + _A_ref(_layernorm(x, axis=-1), A_mem0, A_Wq, A_Wk, A_Wv, A_Wo, A_seg_len)
    x = x + _B_ref(_layernorm(x, axis=-1), B_wqkv, B_w_phi, B_wo)
    x = x + _A_ref(_layernorm(x, axis=-1), A_mem0, A_Wq, A_Wk, A_Wv, A_Wo, A_seg_len)
    x = x + _B_ref(_layernorm(x, axis=-1), B_wqkv, B_w_phi, B_wo)
    return x
```

```python
import functools

import jax
import jax.numpy as jnp
import jax.experimental.pallas as pl
import jax.experimental.pallas.tpu as pltpu

f32, bf16, u32, i32 = jnp.float32, jnp.bfloat16, jnp.uint32, jnp.int32

S, D = 2048, 640
H, DH = 32, 192
M, SEG = 8, 32
L = M + SEG
NSEG = S // SEG
NP = H // 2
PW = 2 * DH
SCALE = DH ** -0.5

F = D // H
NG, GH = 4, 8
GW = F * GH
TB = 512

LAG_S, LAG_PV, LAG_O = 1, 2, 4


def _nn(a, b):
    return jax.lax.dot_general(a, b, (((1,), (0,)), ((), ())), preferred_element_type=f32)


def _nt(a, b):
    return jax.lax.dot_general(a, b, (((1,), (1,)), ((), ())), preferred_element_type=f32)


def _tn(a, b):
    return jax.lax.dot_general(a, b, (((0,), (0,)), ((), ())), preferred_element_type=f32)


def _iota(shape, dim):
    return jax.lax.broadcasted_iota(i32, shape, dim)


def _onehot(cond):
    return jnp.where(cond, 1.0, 0.0).astype(bf16)


def _layernorm(x):
    xc = x - jnp.mean(x, axis=1, keepdims=True)
    var = jnp.mean(xc * xc, axis=1, keepdims=True)
    return xc * jax.lax.rsqrt(var + 1e-5)


def _a_step(s, x_ref, h_ref, wqkv_ref, wo_ref):
    lo = _iota((L, 128), 1) < 64
    lane, row = _iota((L, 128), 1), _iota((L, 128), 0)
    is_a = lane < L
    is_b = (lane >= L) & (lane < 2 * L)
    mask = (row < M) | (row >= jnp.where(is_a, lane, lane - L))
    h = h_ref[...]
    zero = jnp.zeros((L, 128), f32)
    qs, ks, vs, ps, os_ = {}, {}, {}, {}, {}
    acc = []

    def block_diag(t):
        t0, t1, t2 = t[:, 0:128], t[:, 128:256], t[:, 256:384]
        top = jnp.concatenate([t0, jnp.where(lo, t1, 0.0), zero], axis=1)
        bot = jnp.concatenate([zero, jnp.where(lo, 0.0, t1), t2], axis=1)
        pad = jnp.zeros((128 - 2 * L, PW), f32)
        return jnp.concatenate([top, bot, pad], axis=0).astype(bf16)

    def do_qkv(p):
        r = _nn(h, pltpu.bitcast(wqkv_ref[p], bf16))
        qs[p], ks[p], vs[p] = r[:, 0:PW], r[:, PW:2 * PW], r[:, 2 * PW:3 * PW]

    def do_scores(p):
        sc = _nt(qs.pop(p), block_diag(ks.pop(p)))
        sc = jnp.where(mask, sc * SCALE, -1e9)
        m_a = jnp.max(jnp.where(is_a, sc, -jnp.inf), axis=1, keepdims=True)
        m_b = jnp.max(jnp.where(is_b, sc, -jnp.inf), axis=1, keepdims=True)
        e = jnp.exp(sc - jnp.where(is_a, m_a, m_b))
        e_a, e_b = jnp.where(is_a, e, 0.0), jnp.where(is_b, e, 0.0)
        l_a = jnp.sum(e_a, axis=1, keepdims=True)
        l_b = jnp.sum(e_b, axis=1, keepdims=True)
        ps[p] = (e_a + e_b) * (1.0 / jnp.where(is_a, l_a, l_b))

    def do_pv(p):
        os_[p] = _nn(ps.pop(p), block_diag(vs.pop(p)))

    def do_out(p):
        r = _nn(os_.pop(p), pltpu.bitcast(wo_ref[p], bf16))
        acc[:] = [acc[0] + r if acc else r]

    for t in range(NP + LAG_O):
        if t < NP:
            do_qkv(t)
        if 0 <= t - LAG_S < NP:
            do_scores(t - LAG_S)
        if 0 <= t - LAG_O < NP:
            do_out(t - LAG_O)
        if 0 <= t - LAG_PV < NP:
            do_pv(t - LAG_PV)

    nxt = pl.multiple_of(jnp.minimum(s + 1, NSEG - 1) * SEG, SEG)
    h_next = _layernorm(x_ref[pl.ds(nxt, SEG), :])
    x_ref[pl.ds(pl.multiple_of(s * SEG, SEG), SEG), :] += acc[0][M:L]
    h_ref[0:M, :] = acc[0][0:M]
    h_ref[M:L, :] = h_next


def _features(p):
    rows = [p[f * GH:(f + 1) * GH] for f in range(F)]
    hi = functools.reduce(jnp.maximum, rows)
    lo = functools.reduce(jnp.minimum, rows)
    out = []
    for e in ([jnp.exp(r - hi) for r in rows], [jnp.exp(lo - r) for r in rows]):
        inv = 1.0 / functools.reduce(jnp.add, e)
        out += [t * inv for t in e]
    return jnp.concatenate(out, axis=0).astype(bf16)


def _b_accumulate(i, x_ref, wb_ref, kv_ref, phiq_ref):
    t0 = pl.multiple_of(i * TB, TB)
    ln = _layernorm(x_ref[pl.ds(t0, TB), :]).astype(bf16)
    for g in range(NG):
        r = _nt(pltpu.bitcast(wb_ref[g], bf16), ln)
        phi_k = _features(r[GW:2 * GW])
        v_aug = jnp.concatenate([r[2 * GW:3 * GW], jnp.ones((GH, TB), f32)], axis=0)
        kv_ref[g] += _nt(v_aug, phi_k)
        phiq_ref[i, g] = pltpu.bitcast(_features(r[0:GW]), u32)


def _b_output(i, x_ref, wob_ref, kv_ref, phiq_ref):
    t0 = pl.multiple_of(i * TB, TB)
    outs = []
    for g in range(NG):
        r = _nn(kv_ref[g], pltpu.bitcast(phiq_ref[i, g], bf16))
        inv = 1.0 / (r[GW:GW + GH] + 1e-6)
        outs += [r[d * GH:(d + 1) * GH] * inv for d in range(F)]
    o = jnp.concatenate(outs, axis=0).astype(bf16)
    x_ref[pl.ds(t0, TB), :] += _tn(o, pltpu.bitcast(wob_ref[...], bf16))


def _prepare_b(wqkv_ref, wphi_ref, wo_ref, wb_ref, wob_ref):
    hk, ck = _iota((H, D), 0), _iota((H, D), 1)
    phi = functools.reduce(
        jnp.add, [_nn(wphi_ref[d], _onehot(ck == hk * F + d)) for d in range(F)])
    row, col = _iota((GW, D), 0), _iota((GW, D), 1)
    spread = _onehot((_iota((GW, F), 0) >> 3) == _iota((GW, F), 1))
    phi_rows = _nn(spread, phi.astype(bf16))
    for g in range(NG):
        first = ((row & 7) + g * GH) * F
        fold = jnp.where((col >= first) & (col < first + F), phi_rows, 0.0).astype(bf16)
        perm = _onehot(col == first + (row >> 3))
        wt = jnp.concatenate([
            _nt(fold, wqkv_ref[:, 0:D]),
            _nt(fold, wqkv_ref[:, D:2 * D]),
            _nt(perm, wqkv_ref[:, 2 * D:3 * D])], axis=0)
        wb_ref[g] = pltpu.bitcast(wt.astype(bf16), u32)
        wob_ref[g * GW // 2:(g + 1) * GW // 2, :] = pltpu.bitcast(
            _nn(perm, wo_ref[...]).astype(bf16), u32)


def _kernel(x_hbm, mem0_ref, wq_hbm, wk_hbm, wv_hbm, wo_hbm, bqkv_hbm, wphi_ref, bwo_hbm,
            out_hbm,
            x_ref, h_ref, wqkv_ref, wo_ref, wb_ref, wob_ref, kv_ref, phiq_ref,
            io_ref, stage_ref, bqkv_ref, bwo_ref, w_sem, sem):
    x_copy = pltpu.make_async_copy(x_hbm, io_ref, sem.at[0])
    bqkv_copy = pltpu.make_async_copy(bqkv_hbm, bqkv_ref, sem.at[1])
    bwo_copy = pltpu.make_async_copy(bwo_hbm, bwo_ref, sem.at[2])

    def w_copy(p, j):
        src = (wq_hbm, wk_hbm, wv_hbm, wo_hbm)[j]
        return pltpu.make_async_copy(src.at[p], stage_ref.at[p, j], w_sem.at[p, j])

    x_copy.start()
    bqkv_copy.start()
    bwo_copy.start()
    for p in range(NP):
        for j in range(4):
            w_copy(p, j).start()

    x_copy.wait()
    x_ref[...] = io_ref[...].astype(f32)
    bqkv_copy.wait()
    bwo_copy.wait()
    _prepare_b(bqkv_ref, wphi_ref, bwo_ref, wb_ref, wob_ref)

    @pl.loop(0, NP)
    def _(p):
        for j in range(3):
            w_copy(p, j).wait()
            wqkv_ref[p, :, j * PW:(j + 1) * PW] = pltpu.bitcast(stage_ref[p, j].T, u32)
        w_copy(p, 3).wait()
        wo_ref[p] = pltpu.bitcast(stage_ref[p, 3], u32)

    @pl.loop(0, 2)
    def _(_):
        h_ref[0:M, :] = mem0_ref[...].astype(f32)
        h_ref[M:L, :] = _layernorm(x_ref[0:SEG, :])
        pl.loop(0, NSEG)(lambda s: _a_step(s, x_ref, h_ref, wqkv_ref, wo_ref))

        kv_ref[...] = jnp.zeros(kv_ref.shape, f32)
        pl.loop(0, S // TB)(lambda i: _b_accumulate(i, x_ref, wb_ref, kv_ref, phiq_ref))
        shape = (GW + GH, 2 * GW)
        same_head = (_iota(shape, 0) & 7) == (_iota(shape, 1) & 7)
        for g in range(NG):
            kv_ref[g] = jnp.where(same_head, kv_ref[g], 0.0)
        pl.loop(0, S // TB)(lambda i: _b_output(i, x_ref, wob_ref, kv_ref, phiq_ref))

    io_ref[...] = x_ref[...].astype(bf16)
    out_copy = pltpu.make_async_copy(io_ref, out_hbm, sem.at[0])
    out_copy.start()
    out_copy.wait()


@functools.partial(jax.jit, static_argnames=("A_seg_len",))
def pallas_interleave_layers__memory_aug_recurrent_mem_tr__linear_kernel_hedgehog__prompt_kernel(
    A_x: jax.Array,
    A_mem0: jax.Array,
    A_Wq: jax.Array,
    A_Wk: jax.Array,
    A_Wv: jax.Array,
    A_Wo: jax.Array,
    A_seg_len: int,
    B_x: jax.Array,
    B_wqkv: jax.Array,
    B_w_phi: jax.Array,
    B_wo: jax.Array,
):
    del B_x
    assert A_x.shape == (1, S, D) and A_mem0.shape == (1, M, D) and A_seg_len == SEG
    assert A_Wq.shape == (D, H, DH) and B_w_phi.shape == (H, F, F)

    def head_major(w):
        return jnp.transpose(w, (1, 2, 0)).reshape(NP, PW, D)

    hbm = pl.BlockSpec(memory_space=pl.ANY)
    vmem = pl.BlockSpec(memory_space=pltpu.VMEM)
    out = pl.pallas_call(
        _kernel,
        out_shape=jax.ShapeDtypeStruct((S, D), bf16),
        in_specs=[hbm, vmem, hbm, hbm, hbm, hbm, hbm, vmem, hbm],
        out_specs=hbm,
        scratch_shapes=[
            pltpu.VMEM((S, D), f32),
            pltpu.VMEM((L, D), f32),
            pltpu.VMEM((NP, D // 2, 3 * PW), u32),
            pltpu.VMEM((NP, PW // 2, D), u32),
            pltpu.VMEM((NG, 3 * GW // 2, D), u32),
            pltpu.VMEM((D // 2, D), u32),
            pltpu.VMEM((NG, GW + GH, 2 * GW), f32),
            pltpu.VMEM((S // TB, NG, GW, TB), u32),
            pltpu.VMEM((S, D), bf16),
            pltpu.VMEM((NP, 4, PW, D), bf16),
            pltpu.VMEM((D, 3 * D), bf16),
            pltpu.VMEM((D, D), bf16),
            pltpu.SemaphoreType.DMA((NP, 4)),
            pltpu.SemaphoreType.DMA((3,)),
        ],
        compiler_params=pltpu.CompilerParams(vmem_limit_bytes=120 * 1024 * 1024),
    )(
        A_x.reshape(S, D),
        A_mem0.reshape(M, D),
        head_major(A_Wq),
        head_major(A_Wk),
        head_major(A_Wv),
        A_Wo.reshape(NP, PW, D),
        B_wqkv,
        jnp.transpose(B_w_phi, (1, 2, 0)),
        B_wo,
    )
    return out.reshape(1, S, D)
```

```python
import functools

import jax
import jax.numpy as jnp
import jax.experimental.pallas as pl
import jax.experimental.pallas.tpu as pltpu

f32, bf16, u32, i32 = jnp.float32, jnp.bfloat16, jnp.uint32, jnp.int32

S, D = 2048, 640
H, DH = 32, 192
M, SEG = 8, 32
L = M + SEG
NSEG = S // SEG
NP = H // 2
PW = 2 * DH
SCALE = DH ** -0.5

F = D // H
NG, GH = 4, 8
GW = F * GH
TB = 512

UNROLL = 2
ORDER = "q0 v1 s1 k0 o5 p3"
AHEAD = 8
NPRE = 2
PREFETCH, LATE = 2, 4


def _nn(a, b):
    return jax.lax.dot_general(a, b, (((1,), (0,)), ((), ())), preferred_element_type=f32)


def _nt(a, b):
    return jax.lax.dot_general(a, b, (((1,), (1,)), ((), ())), preferred_element_type=f32)


def _tn(a, b):
    return jax.lax.dot_general(a, b, (((0,), (0,)), ((), ())), preferred_element_type=f32)


def _iota(shape, dim):
    return jax.lax.broadcasted_iota(i32, shape, dim)


def _onehot(cond):
    return jnp.where(cond, 1.0, 0.0).astype(bf16)


def _layernorm(x):
    xc = x - jnp.mean(x, axis=1, keepdims=True)
    var = jnp.mean(xc * xc, axis=1, keepdims=True)
    return xc * jax.lax.rsqrt(var + 1e-5)


def _a_segment(s, mem, tok, wqkv_ref, wo_ref, pre_ref):
    head = SEG - AHEAD
    lane, row = _iota((L, 128), 1), _iota((L, 128), 0)
    lo = lane < 64
    is_a = lane < L
    is_b = (lane >= L) & (lane < 2 * L)

    def position(i):
        return jnp.where(i < head, i + M, jnp.where(i < head + M, i - head, i))

    q_pos, k_pos = position(row), position(jnp.where(is_a, lane, lane - L))
    mask = (q_pos < M) | (q_pos >= k_pos)
    h = jnp.concatenate([tok[0:head], mem, tok[head:SEG]], axis=0)
    zero = jnp.zeros((L, 128), f32)
    qs, ks, vs, ps, os_ = {}, {}, {}, {}, {}
    acc = []

    def block_diag(t):
        t0, t1, t2 = t[:, 0:128], t[:, 128:256], t[:, 256:384]
        top = jnp.concatenate([t0, jnp.where(lo, t1, 0.0), zero], axis=1)
        bot = jnp.concatenate([zero, jnp.where(lo, 0.0, t1), t2], axis=1)
        pad = jnp.zeros((128 - 2 * L, PW), f32)
        return jnp.concatenate([top, bot, pad], axis=0).astype(bf16)

    def project(p, j):
        w = pltpu.bitcast(wqkv_ref[p, :, j * PW:(j + 1) * PW], bf16)
        if j >= NPRE:
            return _nn(h, w)
        ahead = pre_ref[p, pl.ds(pl.multiple_of(s * AHEAD, AHEAD), AHEAD), j * PW:(j + 1) * PW]
        return jnp.concatenate([_nn(h[0:L - AHEAD], w), ahead], axis=0)

    def do_q(p):
        qs[p] = project(p, 0)

    def do_k(p):
        ks[p] = project(p, 1)

    def do_v(p):
        vs[p] = project(p, 2)

    def do_scores(p):
        sc = _nt(qs.pop(p), block_diag(ks.pop(p)))
        sc = jnp.where(mask, sc * SCALE, -1e9)
        m_a = jnp.max(jnp.where(is_a, sc, -jnp.inf), axis=1, keepdims=True)
        m_b = jnp.max(jnp.where(is_b, sc, -jnp.inf), axis=1, keepdims=True)
        e = jnp.exp(sc - jnp.where(is_a, m_a, m_b))
        e_a, e_b = jnp.where(is_a, e, 0.0), jnp.where(is_b, e, 0.0)
        l_a = jnp.sum(e_a, axis=1, keepdims=True)
        l_b = jnp.sum(e_b, axis=1, keepdims=True)
        ps[p] = (e_a + e_b) * (1.0 / jnp.where(is_a, l_a, l_b))

    def do_pv(p):
        os_[p] = _nn(ps.pop(p), block_diag(vs.pop(p)))

    def do_out(p):
        o = os_.pop(p)
        o = jnp.concatenate([o[head:head + M], o[0:head], o[head + M:L]], axis=0)
        r = _nn(o, pltpu.bitcast(wo_ref[p], bf16))
        acc[:] = [acc[0] + r if acc else r]

    stages = dict(q=do_q, k=do_k, v=do_v, s=do_scores, p=do_pv, o=do_out)
    order = [(w[0], int(w[1:])) for w in ORDER.split()]
    for t in range(NP + max(lag for _, lag in order)):
        for name, lag in order:
            if 0 <= t - lag < NP:
                stages[name](t - lag)
    return acc[0][0:M], acc[0][M:L]


def _a_step(i, x_ref, h_ref, wqkv_ref, wo_ref, pre_ref):
    mem, tok = h_ref[0:M, :], h_ref[M:L, :]
    for u in range(UNROLL):
        s = i * UNROLL + u
        nxt = pl.multiple_of(jnp.minimum(s + 1, NSEG - 1) * SEG, SEG)
        tok_next = _layernorm(x_ref[pl.ds(nxt, SEG), :])
        mem, out = _a_segment(s, mem, tok, wqkv_ref, wo_ref, pre_ref)
        x_ref[pl.ds(pl.multiple_of(s * SEG, SEG), SEG), :] += out
        tok = tok_next
    h_ref[0:M, :] = mem
    h_ref[M:L, :] = tok


def _features(p):
    rows = [p[f * GH:(f + 1) * GH] for f in range(F)]
    hi = functools.reduce(jnp.maximum, rows)
    lo = functools.reduce(jnp.minimum, rows)
    out = []
    for e in ([jnp.exp(r - hi) for r in rows], [jnp.exp(lo - r) for r in rows]):
        inv = 1.0 / functools.reduce(jnp.add, e)
        out += [t * inv for t in e]
    return jnp.concatenate(out, axis=0).astype(bf16)


def _b_accumulate(i, x_ref, wb_ref, kv_ref, phiq_ref):
    t0 = pl.multiple_of(i * TB, TB)
    ln = _layernorm(x_ref[pl.ds(t0, TB), :]).astype(bf16)
    for g in range(NG):
        r = _nt(pltpu.bitcast(wb_ref[g], bf16), ln)
        phi_k = _features(r[GW:2 * GW])
        v_aug = jnp.concatenate([r[2 * GW:3 * GW], jnp.ones((GH, TB), f32)], axis=0)
        kv_ref[g] += _nt(v_aug, phi_k)
        phiq_ref[i, g] = pltpu.bitcast(_features(r[0:GW]), u32)


def _b_output(i, x_ref, wob_ref, kv_ref, phiq_ref):
    t0 = pl.multiple_of(i * TB, TB)
    outs = []
    for g in range(NG):
        r = _nn(kv_ref[g], pltpu.bitcast(phiq_ref[i, g], bf16))
        inv = 1.0 / (r[GW:GW + GH] + 1e-6)
        outs += [r[d * GH:(d + 1) * GH] * inv for d in range(F)]
    o = jnp.concatenate(outs, axis=0).astype(bf16)
    x = x_ref[pl.ds(t0, TB), :] + _tn(o, pltpu.bitcast(wob_ref[...], bf16))
    x_ref[pl.ds(t0, TB), :] = x
    return x


def _prepare_b(wqkv_ref, wphi_ref, wo_ref, wb_ref, wob_ref, between):
    hk, ck = _iota((H, D), 0), _iota((H, D), 1)
    phi = functools.reduce(
        jnp.add, [_nn(wphi_ref[d], _onehot(ck == hk * F + d)) for d in range(F)])
    spread = _onehot((_iota((GW, F), 0) >> 3) == _iota((GW, F), 1))
    phi_rows = _nn(spread, phi.astype(bf16))
    for g in range(NG):
        between(g)
        c0, cw = g * 128, 256
        row, col = _iota((GW, cw), 0), _iota((GW, cw), 1) + c0
        first = ((row & 7) + g * GH) * F
        fold = jnp.where((col >= first) & (col < first + F),
                         phi_rows[:, c0:c0 + cw], 0.0).astype(bf16)
        perm = _onehot(col == first + (row >> 3))
        wt = jnp.concatenate([
            _nt(fold, wqkv_ref[:, c0:c0 + cw]),
            _nt(fold, wqkv_ref[:, D + c0:D + c0 + cw]),
            _nt(perm, wqkv_ref[:, 2 * D + c0:2 * D + c0 + cw])], axis=0)
        wb_ref[g] = pltpu.bitcast(wt.astype(bf16), u32)
        wob_ref[g * GW // 2:(g + 1) * GW // 2, :] = pltpu.bitcast(
            _nn(perm, wo_ref[c0:c0 + cw, :]).astype(bf16), u32)


def _kernel(x_hbm, mem0_ref, wq_hbm, wk_hbm, wv_hbm, wo_hbm, bqkv_hbm, wphi_ref, bwo_hbm,
            out_hbm,
            x_ref, h_ref, wqkv_ref, wo_ref, pre_ref, tail_ref, wb_ref, wob_ref, kv_ref, phiq_ref,
            io_ref, tail_in_ref, stage_ref, bqkv_ref, bwo_ref, w_sem, sem, out_sem):
    tail_copy = pltpu.make_async_copy(x_hbm.at[:, SEG // AHEAD - 1], tail_in_ref, sem.at[3])
    x_copy = pltpu.make_async_copy(x_hbm, io_ref, sem.at[0])
    bqkv_copy = pltpu.make_async_copy(bqkv_hbm, bqkv_ref, sem.at[1])
    bwo_copy = pltpu.make_async_copy(bwo_hbm, bwo_ref, sem.at[2])

    def w_copy(p, j):
        src = (wq_hbm, wk_hbm, wv_hbm, wo_hbm)[j]
        return pltpu.make_async_copy(src.at[p], stage_ref.at[p, j], w_sem.at[p, j])

    def install(p, j):
        if j < 3:
            wqkv_ref[p, :, j * PW:(j + 1) * PW] = pltpu.bitcast(stage_ref[p, j].T, u32)
        else:
            wo_ref[p] = pltpu.bitcast(stage_ref[p, j], u32)

    early, late = range(NPRE), range(NPRE, 4)
    tail_copy.start()
    for j in early:
        w_copy(0, j).start()
    tail_copy.wait()
    for p in range(1, PREFETCH):
        for j in early:
            w_copy(p, j).start()
    tail_ref[...] = _layernorm(
        tail_in_ref[...].astype(f32).reshape(NSEG * AHEAD, D)).astype(bf16)

    def load_pair(p, install_late):
        @pl.when(p + PREFETCH < NP)
        def _():
            for j in early:
                w_copy(p + PREFETCH, j).start()

        @pl.when(p - LATE + PREFETCH >= 0)
        def _():
            for j in late:
                w_copy(p - LATE + PREFETCH, j).start()

        for when, copy in ((0, bqkv_copy), (1, bwo_copy), (NP - 1, x_copy)):
            pl.when(p == when)(copy.start)
        for j in early:
            w_copy(p, j).wait()
        if install_late:
            for j in late:
                w_copy(p - LATE, j).wait()
        for j in early:
            pre_ref[p, :, j * PW:(j + 1) * PW] = _nt(tail_ref[...], stage_ref[p, j])
            install(p, j)
        if install_late:
            for j in late:
                install(p - LATE, j)

    def install_rest(g):
        for p in range(NP - LATE + g, NP, NG):
            for j in late:
                w_copy(p, j).wait()
            for j in late:
                install(p, j)

    with jax.named_scope("load"):
        pl.loop(0, LATE)(lambda p: load_pair(p, False))
        pl.loop(LATE, NP)(lambda p: load_pair(p, True))
    with jax.named_scope("bprep"):
        for p in range(NP - LATE + PREFETCH, NP):
            for j in late:
                w_copy(p, j).start()
        bqkv_copy.wait()
        bwo_copy.wait()
        _prepare_b(bqkv_ref, wphi_ref, bwo_ref, wb_ref, wob_ref, install_rest)
        x_copy.wait()
        x_ref[...] = io_ref[...].astype(f32).reshape(S, D)

    def out_copy(i):
        rows = pl.ds(i * (TB // SEG), TB // SEG)
        return pltpu.make_async_copy(io_ref.at[rows], out_hbm.at[rows], out_sem.at[i])

    @pl.loop(0, 2)
    def _(layer):
        h_ref[0:M, :] = mem0_ref[...].astype(f32)
        h_ref[M:L, :] = _layernorm(x_ref[0:SEG, :])
        with jax.named_scope("A"):
            pl.loop(0, NSEG // UNROLL)(lambda s: _a_step(s, x_ref, h_ref, wqkv_ref, wo_ref, pre_ref))

        kv_ref[...] = jnp.zeros(kv_ref.shape, f32)
        with jax.named_scope("B1"):
            pl.loop(0, S // TB)(lambda i: _b_accumulate(i, x_ref, wb_ref, kv_ref, phiq_ref))
        shape = (GW + GH, 2 * GW)
        same_head = (_iota(shape, 0) & 7) == (_iota(shape, 1) & 7)
        for g in range(NG):
            kv_ref[g] = jnp.where(same_head, kv_ref[g], 0.0)

        with jax.named_scope("B2"):
            @pl.loop(0, S // TB)
            def _(i):
                x = _b_output(i, x_ref, wob_ref, kv_ref, phiq_ref)
                x = x.reshape(TB // SEG, SEG // AHEAD, AHEAD, D)
                n = TB // SEG * AHEAD
                tail_ref[pl.ds(pl.multiple_of(i * n, n), n), :] = _layernorm(
                    x[:, -1].reshape(n, D)).astype(bf16)
                io_ref[pl.ds(i * (TB // SEG), TB // SEG)] = x.astype(bf16)
                pl.when(layer == 1)(out_copy(i).start)

        with jax.named_scope("pre"):
            @pl.when(layer == 0)
            def _():
                @pl.loop(0, NP)
                def _(p):
                    pre_ref[p] = _nn(
                        tail_ref[...], pltpu.bitcast(wqkv_ref[p, :, 0:NPRE * PW], bf16))

    for i in range(S // TB):
        out_copy(i).wait()


@functools.partial(jax.jit, static_argnames=("A_seg_len",))
def pallas_interleave_layers__memory_aug_recurrent_mem_tr__linear_kernel_hedgehog__prompt_kernel(
    A_x: jax.Array,
    A_mem0: jax.Array,
    A_Wq: jax.Array,
    A_Wk: jax.Array,
    A_Wv: jax.Array,
    A_Wo: jax.Array,
    A_seg_len: int,
    B_x: jax.Array,
    B_wqkv: jax.Array,
    B_w_phi: jax.Array,
    B_wo: jax.Array,
):
    del B_x
    assert A_x.shape == (1, S, D) and A_mem0.shape == (1, M, D) and A_seg_len == SEG
    assert A_Wq.shape == (D, H, DH) and B_w_phi.shape == (H, F, F)

    def head_major(w):
        return jnp.transpose(w, (1, 2, 0)).reshape(NP, PW, D)

    x_blocks = (NSEG, SEG // AHEAD, AHEAD, D)
    hbm = pl.BlockSpec(memory_space=pl.ANY)
    vmem = pl.BlockSpec(memory_space=pltpu.VMEM)
    out = pl.pallas_call(
        _kernel,
        out_shape=jax.ShapeDtypeStruct(x_blocks, bf16),
        in_specs=[hbm, vmem, hbm, hbm, hbm, hbm, hbm, vmem, hbm],
        out_specs=hbm,
        scratch_shapes=[
            pltpu.VMEM((S, D), f32),
            pltpu.VMEM((L, D), f32),
            pltpu.VMEM((NP, D // 2, 3 * PW), u32),
            pltpu.VMEM((NP, PW // 2, D), u32),
            pltpu.VMEM((NP, NSEG * AHEAD, NPRE * PW), f32),
            pltpu.VMEM((NSEG * AHEAD, D), bf16),
            pltpu.VMEM((NG, 3 * GW // 2, D), u32),
            pltpu.VMEM((D // 2, D), u32),
            pltpu.VMEM((NG, GW + GH, 2 * GW), f32),
            pltpu.VMEM((S // TB, NG, GW, TB), u32),
            pltpu.VMEM(x_blocks, bf16),
            pltpu.VMEM((NSEG, AHEAD, D), bf16),
            pltpu.VMEM((NP, 4, PW, D), bf16),
            pltpu.VMEM((D, 3 * D), bf16),
            pltpu.VMEM((D, D), bf16),
            pltpu.SemaphoreType.DMA((NP, 4)),
            pltpu.SemaphoreType.DMA((4,)),
            pltpu.SemaphoreType.DMA((S // TB,)),
        ],
        compiler_params=pltpu.CompilerParams(vmem_limit_bytes=120 * 1024 * 1024),
    )(
        A_x.reshape(x_blocks),
        A_mem0.reshape(M, D),
        head_major(A_Wq),
        head_major(A_Wk),
        head_major(A_Wv),
        A_Wo.reshape(NP, PW, D),
        B_wqkv,
        jnp.transpose(B_w_phi, (1, 2, 0)),
        B_wo,
    )
    return out.reshape(1, S, D)
```

```python
import functools

import jax
import jax.numpy as jnp
import jax.experimental.pallas as pl
import jax.experimental.pallas.tpu as pltpu

f32, bf16, u32, i32 = jnp.float32, jnp.bfloat16, jnp.uint32, jnp.int32

S, D = 2048, 640
H, DH = 32, 192
M, SEG = 8, 32
L = M + SEG
NSEG = S // SEG
NP = H // 2
PW = 2 * DH
SCALE = DH ** -0.5
LOG2E = 1.4426950408889634

F = D // H
PF = 2 * F
NG, GP = 4, 4
GW = PF * GP
TB, SUB = 512, 128

UNROLL = 2
NV = "1111111111111111"
PACK = 3
STASH = 0
FLAGS = None
FLAGS = None
ORDER = "qvqvqv s x kokokooo y p"
LAGS = "q0 k0 v1 s1 x1 y2 p3 o6"
AHEAD = 8
NPRE = 2
PREFETCH, LATE = 2, 4


def _nn(a, b):
    return jax.lax.dot_general(a, b, (((1,), (0,)), ((), ())), preferred_element_type=f32)


def _nt(a, b):
    return jax.lax.dot_general(a, b, (((1,), (1,)), ((), ())), preferred_element_type=f32)


def _tn(a, b):
    return jax.lax.dot_general(a, b, (((0,), (0,)), ((), ())), preferred_element_type=f32)


def _iota(shape, dim):
    return jax.lax.broadcasted_iota(i32, shape, dim)


def _onehot(cond):
    return jnp.where(cond, 1.0, 0.0).astype(bf16)


def _recip(x):
    r = pl.reciprocal(x, approx=True)
    return r * (2.0 - x * r)


def _layernorm(x):
    xc = x - jnp.mean(x, axis=1, keepdims=True)
    var = jnp.mean(xc * xc, axis=1, keepdims=True)
    return xc * jax.lax.rsqrt(var + 1e-5)


def _a_segment(s, mem, tok, wqkv_ref, wo_ref, pre_ref, proj_ref):
    head = SEG - AHEAD
    lane, row = _iota((L, 128), 1), _iota((L, 128), 0)
    lo = lane < 64
    lo8, row8 = _iota((8, 128), 1) < 64, _iota((8, 128), 0)

    def position(i):
        return jnp.where(i < head, i + M, jnp.where(i < head + M, i - head, i))

    q_pos, k_pos = position(row), position(jnp.where(lane < L, lane, lane - L))
    visible = jnp.where((q_pos < M) | (q_pos >= k_pos), 1, 0)
    h = jnp.concatenate([tok[0:head], mem, tok[head:SEG]], axis=0)
    h_now = h[0:L - AHEAD].astype(bf16 if PACK & 1 else f32)
    zero = jnp.zeros((L, 128), f32)
    proj = [{}, {}, {}]
    ps, es, o_mxu, o_vpu = {}, {}, {}, {}
    acc = {}

    def tiles(t):
        return [t[:, c:c + 128] for c in range(0, PW, 128)]

    def bands(top, bot):
        return jnp.concatenate([jnp.concatenate(top, axis=1), jnp.concatenate(bot, axis=1),
                                jnp.zeros((128 - 2 * L, PW), f32)], axis=0).astype(bf16)

    def packed(t):
        return t.astype(bf16) if PACK & 2 and t.shape[0] % 16 == 0 else t

    parts = {}

    def project(p, j, n):
        cols = slice(j * PW + n * 128, j * PW + (n + 1) * 128)
        w = pltpu.bitcast(wqkv_ref[p, :, cols], bf16)
        if j >= NPRE:
            r = _nn(h, w)
        else:
            ahead = pre_ref[p, pl.ds(pl.multiple_of(s * AHEAD, AHEAD), AHEAD), cols]
            r = jnp.concatenate([_nn(h_now, w), ahead], axis=0)
        if STASH >> j & 1:
            proj_ref[p, j, :, n * 128:(n + 1) * 128] = r
            proj[j][p] = proj_ref.at[p, j]
        else:
            parts[p, j, n] = r
            if n == 2:
                proj[j][p] = jnp.concatenate([parts[p, j, i] for i in range(3)], axis=1)

    def do_scores(p):
        r0 = 8 * int(NV[p])
        key = _iota((L - r0, 128), 1)
        is_a, is_b = key < L, (key >= L) & (key < 2 * L)
        k0, k1, k2 = tiles(proj[1][p][...])
        sc = _nt(packed(proj[0][p][r0:L]), bands([k0, jnp.where(lo, k1, 0.0), zero],
                                                 [zero, jnp.where(lo, 0.0, k1), k2]))
        sc = jnp.where(visible[r0:L] > 0, sc * (SCALE * LOG2E), -1e9 * LOG2E)
        m_a = jnp.max(jnp.where(is_a, sc, -jnp.inf), axis=1, keepdims=True)
        m_b = jnp.max(jnp.where(is_b, sc, -jnp.inf), axis=1, keepdims=True)
        e = jnp.exp2(sc - jnp.where(is_a, m_a, m_b))
        e_a, e_b = jnp.where(is_a, e, 0.0), jnp.where(is_b, e, 0.0)
        l_a = jnp.sum(e_a, axis=1, keepdims=True)
        l_b = jnp.sum(e_b, axis=1, keepdims=True)
        ps[p] = (e_a + e_b) * _recip(jnp.where(is_a, l_a, l_b))

    def do_pv(p):
        v = tiles(proj[2][p][...])
        o_mxu[p] = _nn(packed(ps.pop(p)), bands([jnp.where(lo, t, 0.0) for t in v],
                                                [jnp.where(lo, 0.0, t) for t in v]))

    def vpu_keys(p):
        nv = int(NV[p])
        return ([(j, range(nv)) for j in range(head, head + M) if nv]
                + [(j, range(j // 8, nv)) for j in range(8 * nv)])

    def key_row(t, j):
        return tiles(jnp.broadcast_to(t[j:j + 1], (8, PW)))

    def do_vpu_scores(p):
        nv = int(NV[p])
        q = []
        for b in range(nv):
            q0, q1, q2 = tiles(proj[0][p][8 * b:8 * b + 8] * (SCALE * LOG2E))
            q.append((q0, jnp.where(lo8, q1, 0.0), jnp.where(lo8, 0.0, q1), q2))
        sc = [{} for _ in range(nv)]
        for j, blocks in vpu_keys(p):
            k0, k1, k2 = key_row(proj[1][p], j)
            for b in blocks:
                q0, q1a, q1b, q2 = q[b]
                t = jnp.where(lo8, jnp.sum(q0 * k0 + q1a * k1, axis=1, keepdims=True),
                              jnp.sum(q1b * k1 + q2 * k2, axis=1, keepdims=True))
                if j < head and j // 8 == b and j % 8:
                    t = jnp.where(row8 >= j % 8, t, -1e9 * LOG2E)
                sc[b][j] = t
        es[p] = sc

    def do_vpu_pv(p):
        sc = es.pop(p)
        m = [functools.reduce(jnp.maximum, t.values()) for t in sc]
        o = [None] * len(sc)
        for j, blocks in vpu_keys(p):
            v = key_row(proj[2][p], j)
            for b in blocks:
                e = jnp.exp2(sc[b][j] - m[b])
                t = [e * x for x in v] + [e]
                o[b] = t if o[b] is None else [x + y for x, y in zip(o[b], t)]
        o_vpu[p] = []
        for t in o:
            inv = _recip(t[3])
            o_vpu[p].append(jnp.concatenate([x * inv for x in t[0:3]], axis=1))

    def do_out(p, n):
        o = jnp.concatenate(o_vpu[p] + [o_mxu[p]], axis=0)
        o = jnp.concatenate([o[head:head + M], o[0:head], o[head + M:L]], axis=0)
        r = _nn(o, pltpu.bitcast(wo_ref[p, :, n * 128:(n + 1) * 128], bf16))
        acc[n] = acc[n] + r if n in acc else r

    stages = dict(q=lambda p, n: project(p, 0, n), k=lambda p, n: project(p, 1, n),
                  v=lambda p, n: project(p, 2, n), o=do_out,
                  s=do_scores, p=do_pv, x=do_vpu_scores, y=do_vpu_pv)
    lag = {w[0]: int(w[1:]) for w in LAGS.split()}
    for t in range(NP + max(lag.values())):
        count = dict(q=0, k=0, v=0, o=0)
        for name in ORDER.replace(" ", ""):
            args = ()
            if name in count:
                args = (count[name],)
                count[name] += 1
            if 0 <= t - lag[name] < NP:
                stages[name](t - lag[name], *args)
    out = jnp.concatenate([acc[n] for n in sorted(acc)], axis=1)
    return out[0:M], out[M:L]


def _store_ln(i, x_ref, ln_ref):
    rows = pl.ds(pl.multiple_of(i * (UNROLL * SEG), UNROLL * SEG), UNROLL * SEG)
    ln_ref[rows, :] = _layernorm(x_ref[rows, :]).astype(bf16)


def _a_step(i, x_ref, h_ref, wqkv_ref, wo_ref, pre_ref, proj_ref, ln_ref):
    _store_ln(jnp.maximum(i - 1, 0), x_ref, ln_ref)
    mem, tok = h_ref[0:M, :], h_ref[M:L, :]
    for u in range(UNROLL):
        s = i * UNROLL + u
        nxt = pl.multiple_of(jnp.minimum(s + 1, NSEG - 1) * SEG, SEG)
        tok_next = _layernorm(x_ref[pl.ds(nxt, SEG), :])
        mem, out = _a_segment(s, mem, tok, wqkv_ref, wo_ref, pre_ref, proj_ref.at[u])
        x_ref[pl.ds(pl.multiple_of(s * SEG, SEG), SEG), :] += out
        tok = tok_next
    h_ref[0:M, :] = mem
    h_ref[M:L, :] = tok


def a_extra_scratch():
    return [pltpu.VMEM((UNROLL, NP, 3, L, PW), f32), pltpu.VMEM((S, D), bf16)]


def _over_features(op, rows):
    t = functools.reduce(op, rows)
    t = op(t, pltpu.roll(t, 4, 0))
    return op(t, pltpu.roll(t, 2, 0))


def _features(p):
    rows = [p[r:r + 8] * LOG2E for r in range(0, PF, 8)]
    hi, lo = _over_features(jnp.maximum, rows), _over_features(jnp.minimum, rows)
    out = []
    for e in ([jnp.exp2(r - hi) for r in rows], [jnp.exp2(lo - r) for r in rows]):
        inv = _recip(_over_features(jnp.add, e))
        out += [t * inv for t in e]
    return jnp.concatenate(out, axis=0).astype(bf16)


def _b_accumulate(i, ln_ref, wb_ref, kv_ref, phiq_ref):
    ln = ln_ref[pl.ds(pl.multiple_of(i * TB, TB), TB), :]
    kv = {}

    def project(g):
        r = _nt(pltpu.bitcast(wb_ref[g], bf16), ln)
        for n in range(GP):
            k, v, q = (r[j * GW + n * PF:j * GW + (n + 1) * PF] for j in range(3))
            kv[g * GP + n] = (jnp.concatenate([v, jnp.ones((8, TB), f32)], axis=0),
                              _features(k))
            phiq_ref[i, g * GP + n] = pltpu.bitcast(_features(q), u32)

    for g in range(NG + 1):
        if g < NG:
            project(g)
        for n in range((g - 1) * GP, g * GP) if g else ():
            kv_ref[n] += _nt(*kv.pop(n))


def _b_output(i, x_ref, wob_ref, kv_ref, phiq_ref):
    o, out = {}, []
    nsub = TB // SUB
    for t in range(nsub + 1):
        if t < nsub:
            rows = []
            for n in range(NP):
                r = _nn(kv_ref[n], pltpu.bitcast(phiq_ref[i, n, :, t * SUB:(t + 1) * SUB], bf16))
                inv = 1.0 / (r[PF:PF + 8] + 1e-6)
                rows += [r[d:d + 8] * inv for d in range(0, PF, 8)]
            o[t] = jnp.concatenate(rows, axis=0).astype(bf16)
        if t:
            tok = pl.ds(pl.multiple_of(i * TB + (t - 1) * SUB, SUB), SUB)
            x = x_ref[tok, :] + _tn(o.pop(t - 1), pltpu.bitcast(wob_ref[...], bf16))
            x_ref[tok, :] = x
            out.append(x)
    return jnp.concatenate(out, axis=0)


def _prepare_b(wqkv_ref, wphi_ref, wo_ref, wb_ref, wob_ref, between):
    hk, ck = _iota((H, D), 0), _iota((H, D), 1)
    phi = functools.reduce(
        jnp.add, [_nn(wphi_ref[d], _onehot(ck == hk * F + d)) for d in range(F)])

    def decode(row):
        pair = sum(jnp.where(row >= n * PF, 1, 0) for n in range(1, GP))
        return (row - pair * PF) >> 1, 2 * pair + (row & 1)

    spread = _onehot(decode(_iota((GW, F), 0))[0] == _iota((GW, F), 1))
    phi_rows = _nn(spread, phi.astype(bf16))
    cw = 256
    feature, head = decode(_iota((GW, cw), 0))
    for g in range(NG):
        between(g)
        c0 = g * 128
        col = _iota((GW, cw), 1) + (c0 - g * GW) - head * F
        fold = jnp.where((col >= 0) & (col < F), phi_rows[:, c0:c0 + cw], 0.0).astype(bf16)
        perm = _onehot(col == feature)
        wt = jnp.concatenate([
            _nt(fold, wqkv_ref[:, D + c0:D + c0 + cw]),
            _nt(perm, wqkv_ref[:, 2 * D + c0:2 * D + c0 + cw]),
            _nt(fold, wqkv_ref[:, c0:c0 + cw])], axis=0)
        wb_ref[g] = pltpu.bitcast(wt.astype(bf16), u32)
        wob_ref[g * GW // 2:(g + 1) * GW // 2, :] = pltpu.bitcast(
            _nn(perm, wo_ref[c0:c0 + cw, :]).astype(bf16), u32)


def _kernel(x_hbm, mem0_ref, wq_hbm, wk_hbm, wv_hbm, wo_hbm, bqkv_hbm, wphi_ref, bwo_hbm,
            out_hbm,
            x_ref, h_ref, wqkv_ref, wo_ref, pre_ref, tail_ref, wb_ref, wob_ref, kv_ref, phiq_ref,
            proj_ref, ln_ref, io_ref, tail_in_ref, stage_ref, bqkv_ref, bwo_ref, w_sem, sem, out_sem):
    tail_copy = pltpu.make_async_copy(x_hbm.at[:, SEG // AHEAD - 1], tail_in_ref, sem.at[3])
    x_copy = pltpu.make_async_copy(x_hbm, io_ref, sem.at[0])
    bqkv_copy = pltpu.make_async_copy(bqkv_hbm, bqkv_ref, sem.at[1])
    bwo_copy = pltpu.make_async_copy(bwo_hbm, bwo_ref, sem.at[2])

    def w_copy(p, j):
        src = (wq_hbm, wk_hbm, wv_hbm, wo_hbm)[j]
        return pltpu.make_async_copy(src.at[p], stage_ref.at[p, j], w_sem.at[p, j])

    def install(p, j):
        w = stage_ref[p, j]
        if j >= 2:
            w = jnp.concatenate(
                [w[r + c:r + c + 64] for c in range(0, DH, 64) for r in (0, DH)], axis=0)
        if j < 3:
            wqkv_ref[p, :, j * PW:(j + 1) * PW] = pltpu.bitcast(w.T, u32)
        else:
            wo_ref[p] = pltpu.bitcast(w, u32)

    early, late = range(NPRE), range(NPRE, 4)
    tail_copy.start()
    for j in early:
        w_copy(0, j).start()
    tail_copy.wait()
    for p in range(1, PREFETCH):
        for j in early:
            w_copy(p, j).start()
    tail_ref[...] = _layernorm(
        tail_in_ref[...].astype(f32).reshape(NSEG * AHEAD, D)).astype(bf16)

    def load_pair(p, install_late):
        @pl.when(p + PREFETCH < NP)
        def _():
            for j in early:
                w_copy(p + PREFETCH, j).start()

        @pl.when(p - LATE + PREFETCH >= 0)
        def _():
            for j in late:
                w_copy(p - LATE + PREFETCH, j).start()

        for when, copy in ((0, bqkv_copy), (1, bwo_copy), (NP - 1, x_copy)):
            pl.when(p == when)(copy.start)
        for j in early:
            w_copy(p, j).wait()
        if install_late:
            for j in late:
                w_copy(p - LATE, j).wait()
        for j in early:
            pre_ref[p, :, j * PW:(j + 1) * PW] = _nt(tail_ref[...], stage_ref[p, j])
            install(p, j)
        if install_late:
            for j in late:
                install(p - LATE, j)

    def install_rest(g):
        for p in range(NP - LATE + g, NP, NG):
            for j in late:
                w_copy(p, j).wait()
            for j in late:
                install(p, j)

    with jax.named_scope("load"):
        pl.loop(0, LATE)(lambda p: load_pair(p, False))
        pl.loop(LATE, NP)(lambda p: load_pair(p, True))
    with jax.named_scope("bprep"):
        for p in range(NP - LATE + PREFETCH, NP):
            for j in late:
                w_copy(p, j).start()
        bqkv_copy.wait()
        bwo_copy.wait()
        _prepare_b(bqkv_ref, wphi_ref, bwo_ref, wb_ref, wob_ref, install_rest)
        x_copy.wait()
        x_ref[...] = io_ref[...].astype(f32).reshape(S, D)

    def out_copy(i):
        rows = pl.ds(i * (TB // SEG), TB // SEG)
        return pltpu.make_async_copy(io_ref.at[rows], out_hbm.at[rows], out_sem.at[i])

    @pl.loop(0, 2)
    def _(layer):
        h_ref[0:M, :] = mem0_ref[...].astype(f32)
        h_ref[M:L, :] = _layernorm(x_ref[0:SEG, :])
        with jax.named_scope("A"):
            pl.loop(0, NSEG // UNROLL)(lambda s: _a_step(s, x_ref, h_ref, wqkv_ref, wo_ref, pre_ref, proj_ref, ln_ref))
        _store_ln(NSEG // UNROLL - 1, x_ref, ln_ref)

        kv_ref[...] = jnp.zeros(kv_ref.shape, f32)
        with jax.named_scope("B1"):
            pl.loop(0, S // TB)(lambda i: _b_accumulate(i, ln_ref, wb_ref, kv_ref, phiq_ref))
        shape = kv_ref.shape[1:]
        same_head = (_iota(shape, 0) & 1) == (_iota(shape, 1) & 1)
        for n in range(NP):
            kv_ref[n] = jnp.where(same_head, kv_ref[n], 0.0)

        with jax.named_scope("B2"):
            @pl.loop(0, S // TB)
            def _(i):
                x = _b_output(i, x_ref, wob_ref, kv_ref, phiq_ref)
                x = x.reshape(TB // SEG, SEG // AHEAD, AHEAD, D)
                n = TB // SEG * AHEAD
                tail_ref[pl.ds(pl.multiple_of(i * n, n), n), :] = _layernorm(
                    x[:, -1].reshape(n, D)).astype(bf16)
                io_ref[pl.ds(i * (TB // SEG), TB // SEG)] = x.astype(bf16)
                pl.when(layer == 1)(out_copy(i).start)

        with jax.named_scope("pre"):
            @pl.when(layer == 0)
            def _():
                @pl.loop(0, NP)
                def _(p):
                    pre_ref[p] = _nn(
                        tail_ref[...], pltpu.bitcast(wqkv_ref[p, :, 0:NPRE * PW], bf16))

    for i in range(S // TB):
        out_copy(i).wait()


@functools.partial(jax.jit, static_argnames=("A_seg_len",))
def pallas_interleave_layers__memory_aug_recurrent_mem_tr__linear_kernel_hedgehog__prompt_kernel(
    A_x: jax.Array,
    A_mem0: jax.Array,
    A_Wq: jax.Array,
    A_Wk: jax.Array,
    A_Wv: jax.Array,
    A_Wo: jax.Array,
    A_seg_len: int,
    B_x: jax.Array,
    B_wqkv: jax.Array,
    B_w_phi: jax.Array,
    B_wo: jax.Array,
):
    del B_x
    assert A_x.shape == (1, S, D) and A_mem0.shape == (1, M, D) and A_seg_len == SEG
    assert A_Wq.shape == (D, H, DH) and B_w_phi.shape == (H, F, F)

    def head_major(w):
        return jnp.transpose(w, (1, 2, 0)).reshape(NP, PW, D)

    x_blocks = (NSEG, SEG // AHEAD, AHEAD, D)
    hbm = pl.BlockSpec(memory_space=pl.ANY)
    vmem = pl.BlockSpec(memory_space=pltpu.VMEM)
    out = pl.pallas_call(
        _kernel,
        out_shape=jax.ShapeDtypeStruct(x_blocks, bf16),
        in_specs=[hbm, vmem, hbm, hbm, hbm, hbm, hbm, vmem, hbm],
        out_specs=hbm,
        scratch_shapes=[
            pltpu.VMEM((S, D), f32),
            pltpu.VMEM((L, D), f32),
            pltpu.VMEM((NP, D // 2, 3 * PW), u32),
            pltpu.VMEM((NP, PW // 2, D), u32),
            pltpu.VMEM((NP, NSEG * AHEAD, NPRE * PW), f32),
            pltpu.VMEM((NSEG * AHEAD, D), bf16),
            pltpu.VMEM((NG, 3 * GW // 2, D), u32),
            pltpu.VMEM((D // 2, D), u32),
            pltpu.VMEM((NP, PF + 8, 2 * PF), f32),
            pltpu.VMEM((S // TB, NP, PF, TB), u32),
            *a_extra_scratch(),
            pltpu.VMEM(x_blocks, bf16),
            pltpu.VMEM((NSEG, AHEAD, D), bf16),
            pltpu.VMEM((NP, 4, PW, D), bf16),
            pltpu.VMEM((D, 3 * D), bf16),
            pltpu.VMEM((D, D), bf16),
            pltpu.SemaphoreType.DMA((NP, 4)),
            pltpu.SemaphoreType.DMA((4,)),
            pltpu.SemaphoreType.DMA((S // TB,)),
        ],
        compiler_params=pltpu.CompilerParams(vmem_limit_bytes=120 * 1024 * 1024, flags=FLAGS),
    )(
        A_x.reshape(x_blocks),
        A_mem0.reshape(M, D),
        head_major(A_Wq),
        head_major(A_Wk),
        head_major(A_Wv),
        A_Wo.reshape(NP, PW, D),
        B_wqkv,
        jnp.transpose(B_w_phi, (1, 2, 0)),
        B_wo,
    )
    return out.reshape(1, S, D)
```

```python
import functools

import jax
import jax.numpy as jnp
import jax.experimental.pallas as pl
import jax.experimental.pallas.tpu as pltpu

f32, bf16, u32, i32 = jnp.float32, jnp.bfloat16, jnp.uint32, jnp.int32

S, D = 2048, 640
H, DH = 32, 192
M, SEG = 8, 32
L = M + SEG
NSEG = S // SEG
NP = H // 2
PW = 2 * DH
LOG2E = 1.4426950408889634
SCALE = DH ** -0.5 * LOG2E
MASKED = -1e9 * LOG2E

AHEAD = 8
HEAD = SEG - AHEAD
UNROLL = 2
ORDER = ("qvqvqvsxkokokooop", "qvqvqvsxkokokooop")
LAGS = ("q0 k0 v1 s1 x1 p3 o6", "q0 k0 v1 s1 x1 p3 o6")
ON_VPU = ("1" * NP, "1" * NP)
PREFETCH, LATE = 4, 4
X_FIRST = 2 * UNROLL

F = D // H
PF = 2 * F
NG, GP = 4, 4
GW = PF * GP
TB, TB2, SUB = 256, 512, 128
FLAGS = None


def _nn(a, b):
    return jax.lax.dot_general(a, b, (((1,), (0,)), ((), ())), preferred_element_type=f32)


def _nt(a, b):
    return jax.lax.dot_general(a, b, (((1,), (1,)), ((), ())), preferred_element_type=f32)


def _tn(a, b):
    return jax.lax.dot_general(a, b, (((0,), (0,)), ((), ())), preferred_element_type=f32)


def _unpack(w):
    return pltpu.bitcast(w, bf16)


def _pack(w):
    return pltpu.bitcast(w.astype(bf16), u32)


def _iota(shape, dim):
    return jax.lax.broadcasted_iota(i32, shape, dim)


def _onehot(cond):
    return jnp.where(cond, 1.0, 0.0).astype(bf16)


def _rows(i, n):
    return pl.ds(pl.multiple_of(i * n, n), n)


def _recip(x):
    r = pl.reciprocal(x, approx=True)
    return r * (2.0 - x * r)


def _layernorm(x):
    xc = x - jnp.mean(x, axis=1, keepdims=True)
    var = jnp.mean(xc * xc, axis=1, keepdims=True)
    return xc * jax.lax.rsqrt(var + 1e-5)


def _store_caps(cap_ref):
    def position(i):
        return jnp.where(i < HEAD, i + M, jnp.where(i < HEAD + M, i - HEAD, i))

    query = position(_iota((L, 128), 0))
    for n in range(2):
        key = _iota((L, 128), 1) - n * L
        cap = jnp.where((query < M) | (query >= position(key)), jnp.inf, MASKED)
        cap_ref[n * L:(n + 1) * L] = jnp.where((key >= 0) & (key < L), cap, -jnp.inf)
    r = _iota((64, 128), 0)
    cap_ref[2 * L:2 * L + 64] = jnp.where((r & 7) >= (r >> 3), jnp.inf, MASKED)


def _a_segment(layer, s, mem, tok, wqkv_ref, wo_ref, pre_ref, cap_ref):
    lo, lo8 = _iota((L, 128), 1) < 64, _iota((8, 128), 1) < 64
    h = jnp.concatenate([tok[0:HEAD], mem, tok[HEAD:SEG]], axis=0)
    h_now = h[0:L - AHEAD].astype(bf16)
    q, k, v, prob, o_mxu, o_vpu, acc = {}, {}, {}, {}, {}, {}, {}

    def bands(top, bot):
        return jnp.concatenate(
            [jnp.concatenate(top, axis=1), jnp.concatenate(bot, axis=1),
             jnp.zeros((128 - 2 * L, 128 * len(top)), f32)], axis=0).astype(bf16)

    def lhs(t):
        return t.astype(bf16) if t.shape[0] % 16 == 0 else t

    def first_mxu_row(p):
        return 8 * int(ON_VPU[layer][p])

    def project(j, p, n):
        cols = slice(j * PW + n * 128, j * PW + (n + 1) * 128)
        w = _unpack(wqkv_ref[p, :, cols])
        if layer == 0 and j < 2:
            r = jnp.concatenate([_nn(h_now, w), pre_ref[p, _rows(s, AHEAD), cols]], axis=0)
        else:
            r = _nn(h, w)
        (q, k, v)[j][p, n] = r

    def scores(p):
        r0 = first_mxu_row(p)
        both = _nt(lhs(q[p, 1][r0:L]),
                   bands([jnp.where(lo, k[p, 1], 0.0)], [jnp.where(lo, 0.0, k[p, 1])]))
        rest = _nt(lhs(jnp.concatenate([q[p, 0][r0:L], q[p, 2][r0:L]], axis=0)),
                   bands([k[p, 0]], [k[p, 2]]))
        out = []
        for n in range(2):
            t = (both + rest[n * (L - r0):(n + 1) * (L - r0)]) * SCALE
            t = jnp.minimum(t, cap_ref[n * L + r0:(n + 1) * L])
            e = jnp.exp2(t - jnp.max(t, axis=1, keepdims=True))
            out.append(e * _recip(jnp.sum(e, axis=1, keepdims=True)))
        prob[p] = out[0] + out[1]

    def mix(p):
        o_mxu[p] = _nn(lhs(prob[p]), bands([jnp.where(lo, v[p, n], 0.0) for n in range(3)],
                                           [jnp.where(lo, 0.0, v[p, n]) for n in range(3)]))

    def attend_on_vpu(p):
        o_vpu[p] = []
        if not first_mxu_row(p):
            return
        q0, q1, q2 = (q[p, n][0:8] * SCALE for n in range(3))
        q1a, q1b = jnp.where(lo8, q1, 0.0), jnp.where(lo8, 0.0, q1)
        keys = list(range(HEAD, HEAD + M)) + list(range(8))

        def row(t, j):
            return [jnp.broadcast_to(t[p, n][j:j + 1], (8, 128)) for n in range(3)]

        sc = {}
        for j in keys:
            k0, k1, k2 = row(k, j)
            t = jnp.where(lo8, jnp.sum(q0 * k0 + q1a * k1, axis=1, keepdims=True),
                          jnp.sum(q1b * k1 + q2 * k2, axis=1, keepdims=True))
            if 0 < j < 8:
                t = jnp.minimum(t, cap_ref[2 * L + 8 * j:2 * L + 8 * j + 8])
            sc[j] = t
        top = functools.reduce(jnp.maximum, sc.values())
        o = None
        for j in keys:
            e = jnp.exp2(sc[j] - top)
            t = [e * x for x in row(v, j)] + [e]
            o = t if o is None else [x + y for x, y in zip(o, t)]
        inv = _recip(o[3])
        o_vpu[p] = [jnp.concatenate([x * inv for x in o[0:3]], axis=1)]

    def output(p, n):
        o = jnp.concatenate(o_vpu[p] + [o_mxu[p]], axis=0)
        o = jnp.concatenate([o[HEAD:HEAD + M], o[0:HEAD], o[HEAD + M:L]], axis=0)
        r = _nn(o, _unpack(wo_ref[p, :, n * 128:(n + 1) * 128]))
        acc[n] = acc[n] + r if n in acc else r

    stages = dict(q=functools.partial(project, 0), k=functools.partial(project, 1),
                  v=functools.partial(project, 2), o=output,
                  s=scores, p=mix, x=attend_on_vpu)
    lag = {w[0]: int(w[1:]) for w in LAGS[layer].split()}
    for t in range(NP + max(lag.values())):
        tile = dict(q=0, k=0, v=0, o=0)
        for name in ORDER[layer]:
            args = ()
            if name in tile:
                args = (tile[name],)
                tile[name] += 1
            if 0 <= t - lag[name] < NP:
                stages[name](t - lag[name], *args)
    out = jnp.concatenate([acc[n] for n in range(D // 128)], axis=1)
    return out[0:M], out[M:L]


def _store_ln(i, x_ref, ln_ref):
    rows = _rows(i, UNROLL * SEG)
    ln_ref[rows, :] = _layernorm(x_ref[rows, :]).astype(bf16)


def _a_steps(layer, i, read_x, x_ref, h_ref, ln_ref, *refs):
    _store_ln(jnp.maximum(i - 1, 0), x_ref, ln_ref)
    mem, tok = h_ref[0:M, :], h_ref[M:L, :]
    for u in range(UNROLL):
        s = i * UNROLL + u
        tok_next = _layernorm(read_x(jnp.minimum(s + 1, NSEG - 1)))
        mem, out = _a_segment(layer, s, mem, tok, *refs)
        x_ref[_rows(s, SEG), :] = read_x(s) + out
        tok = tok_next
    h_ref[0:M, :] = mem
    h_ref[M:L, :] = tok


def _over_features(op, rows):
    t = functools.reduce(op, rows)
    t = op(t, pltpu.roll(t, 4, 0))
    return op(t, pltpu.roll(t, 2, 0))


def _features(p):
    rows = [p[r:r + 8] * LOG2E for r in range(0, PF, 8)]
    hi, lo = _over_features(jnp.maximum, rows), _over_features(jnp.minimum, rows)
    out = []
    for e in ([jnp.exp2(r - hi) for r in rows], [jnp.exp2(lo - r) for r in rows]):
        inv = _recip(_over_features(jnp.add, e))
        out += [t * inv for t in e]
    return jnp.concatenate(out, axis=0).astype(bf16)


def _b_accumulate(i, ln_ref, wb_ref, kv_ref, phiq_ref):
    ln = ln_ref[_rows(i, TB), :]
    kv = {}
    for g in range(NG + 1):
        if g < NG:
            r = _nt(_unpack(wb_ref[g]), ln)
            for n in range(GP):
                k, v, q = (r[j * GW + n * PF:j * GW + (n + 1) * PF] for j in range(3))
                kv[g * GP + n] = (jnp.concatenate([v, jnp.ones((8, TB), f32)], axis=0),
                                  _features(k))
                phi_q = _pack(_features(q))
                for t in range(TB // SUB):
                    phiq_ref[i * (TB // SUB) + t, g * GP + n] = phi_q[:, t * SUB:(t + 1) * SUB]
        for n in range((g - 1) * GP, g * GP) if g else ():
            kv_ref[n] += _nt(*kv.pop(n))


def _b_mask(kv_ref):
    row, col = _iota((PF + 8, 2 * PF), 0), _iota((PF + 8, 2 * PF), 1)
    head = jnp.where(((row >= F) & (row < PF)) | (row >= PF + 4), 1, 0)
    for n in range(NP):
        kv_ref[n] = jnp.where(head == (col & 1), kv_ref[n], 0.0)


def _b_output(i, x_ref, io_ref, wob_ref, kv_ref, phiq_ref):
    o = {}
    nsub = TB2 // SUB
    for t in range(nsub + 1):
        if t < nsub:
            rows = []
            for n in range(NP):
                r = _nn(kv_ref[n], _unpack(phiq_ref[i * nsub + t, n]))
                inv = 1.0 / (r[PF:PF + 8] + 1e-6)
                a, b = (jnp.broadcast_to(inv[j:j + 1], inv.shape) for j in (0, 4))
                rows += [r[8 * j:8 * j + 8] * c for j, c in enumerate((a, a, inv, b, b))]
            o[t] = jnp.concatenate(rows, axis=0).astype(bf16)
        if t:
            blk = i * nsub + t - 1
            x = x_ref[_rows(blk, SUB), :] + _tn(o.pop(t - 1), _unpack(wob_ref[...]))
            x_ref[_rows(blk, SUB), :] = x
            io_ref[_rows(blk, SUB), :] = x.astype(bf16)


def _prepare_b(wqkv_ref, wphi_ref, wo_ref, wb_ref, wob_ref):
    hk, ck = _iota((H, D), 0), _iota((H, D), 1)
    phi = functools.reduce(
        jnp.add, [_nn(wphi_ref[d], _onehot(ck == hk * F + d)) for d in range(F)])

    def decode(row):
        pair = sum(jnp.where(row >= n * PF, 1, 0) for n in range(1, GP))
        return (row - pair * PF) >> 1, 2 * pair + (row & 1)

    spread = _onehot(decode(_iota((GW, F), 0))[0] == _iota((GW, F), 1))
    phi_rows = _nn(spread, phi.astype(bf16))
    cw = 256
    col = _iota((GW, cw), 1) - decode(_iota((GW, cw), 0))[1] * F
    wv = _pack(wqkv_ref[:, 2 * D:3 * D].T)
    for g in range(NG):
        c0 = g * 128
        d = col + (c0 - g * GW)
        fold = jnp.where((d >= 0) & (d < F), phi_rows[:, c0:c0 + cw], 0.0).astype(bf16)
        half = GW // 2
        wb_ref[g, 0:half] = _pack(_nt(fold, wqkv_ref[:, D + c0:D + c0 + cw]))
        wb_ref[g, half:2 * half] = wv[g * half:(g + 1) * half]
        wb_ref[g, 2 * half:3 * half] = _pack(_nt(fold, wqkv_ref[:, c0:c0 + cw]))
    wob_ref[...] = _pack(wo_ref[...])


def _kernel(x_hbm, x_tiles_hbm, mem0_ref, wq_hbm, wk_hbm, wv_hbm, wo_hbm,
            bqkv_hbm, wphi_ref, bwo_hbm, out_hbm,
            x_ref, h_ref, ln_ref, wqkv_ref, wo_ref, pre_ref, cap_ref,
            wb_ref, wob_ref, kv_ref, phiq_ref,
            io_ref, tail_in_ref, tail_ref, stage_ref, bqkv_ref, bwo_ref, w_sem, sem, out_sem):
    first, rest = pl.ds(0, X_FIRST * SEG), pl.ds(X_FIRST * SEG, S - X_FIRST * SEG)
    x_first = pltpu.make_async_copy(x_hbm.at[first], io_ref.at[first], sem.at[0])
    x_rest = pltpu.make_async_copy(x_hbm.at[rest], io_ref.at[rest], sem.at[1])
    tail_copy = pltpu.make_async_copy(
        x_tiles_hbm.at[:, SEG // AHEAD - 1], tail_in_ref, sem.at[2])
    bqkv_copy = pltpu.make_async_copy(bqkv_hbm, bqkv_ref, sem.at[3])
    bwo_copy = pltpu.make_async_copy(bwo_hbm, bwo_ref, sem.at[4])

    def w_copy(p, j):
        src = (wq_hbm, wk_hbm, wv_hbm, wo_hbm)[j]
        return pltpu.make_async_copy(src.at[p], stage_ref.at[p, j], w_sem.at[p, j])

    def install(p, j):
        w = stage_ref[p, j]
        if j >= 2:
            w = jnp.concatenate(
                [w[r + c:r + c + 64] for c in range(0, DH, 64) for r in (0, DH)], axis=0)
        if j < 3:
            wqkv_ref[p, :, j * PW:(j + 1) * PW] = _pack(w.T)
        else:
            wo_ref[p] = _pack(w)

    early, late = (0, 1), (2, 3)
    tail_copy.start()
    w_copy(0, 0).start()
    _store_caps(cap_ref)
    tail_copy.wait()
    w_copy(0, 1).start()
    for p in range(1, PREFETCH):
        for j in early:
            w_copy(p, j).start()
    tail_ref[...] = _layernorm(
        tail_in_ref[...].astype(f32).reshape(NSEG * AHEAD, D)).astype(bf16)

    def load_pair(p, install_late):
        for j in early:
            w_copy(p, j).wait()
        if install_late:
            for j in late:
                w_copy(p - LATE, j).wait()

        @pl.when(p + PREFETCH < NP)
        def _():
            for j in early:
                w_copy(p + PREFETCH, j).start()

        for j in late:
            w_copy(p, j).start()
        for j in early:
            pre_ref[p, :, j * PW:(j + 1) * PW] = _nt(tail_ref[...], stage_ref[p, j])
            install(p, j)
        if install_late:
            for j in late:
                install(p - LATE, j)

    with jax.named_scope("load"):
        pl.loop(0, LATE)(lambda p: load_pair(p, False))
        bqkv_copy.start()
        bwo_copy.start()
        x_first.start()
        pl.loop(LATE, NP)(lambda p: load_pair(p, True))
    with jax.named_scope("bprep"):
        bqkv_copy.wait()
        bwo_copy.wait()
        _prepare_b(bqkv_ref, wphi_ref, bwo_ref, wb_ref, wob_ref)

        @pl.loop(NP - LATE, NP)
        def _(p):
            for j in late:
                w_copy(p, j).wait()
                install(p, j)
        x_first.wait()
        x_rest.start()
        x_ref[0:UNROLL * SEG, :] = io_ref[0:UNROLL * SEG, :].astype(f32)

    def out_copy(i):
        rows = _rows(i, TB2)
        return pltpu.make_async_copy(io_ref.at[rows], out_hbm.at[rows], out_sem.at[i])

    def layer_a(layer):
        def read_x(s):
            return (x_ref if layer else io_ref)[_rows(s, SEG), :].astype(f32)

        h_ref[0:M, :] = mem0_ref[...].astype(f32)
        h_ref[M:L, :] = _layernorm(x_ref[0:SEG, :])

        @pl.loop(0, NSEG // UNROLL)
        def _(i):
            if layer == 0:
                pl.when(i == 1)(x_rest.wait)
            _a_steps(layer, i, read_x, x_ref, h_ref, ln_ref, wqkv_ref, wo_ref, pre_ref, cap_ref)

    @pl.loop(0, 2)
    def _(block):
        with jax.named_scope("A"):
            for layer in range(2):
                pl.when(block == layer)(functools.partial(layer_a, layer))
        _store_ln(NSEG // UNROLL - 1, x_ref, ln_ref)
        kv_ref[...] = jnp.zeros(kv_ref.shape, f32)
        with jax.named_scope("B1"):
            pl.loop(0, S // TB)(lambda i: _b_accumulate(i, ln_ref, wb_ref, kv_ref, phiq_ref))
        _b_mask(kv_ref)
        with jax.named_scope("B2"):
            @pl.loop(0, S // TB2)
            def _(i):
                _b_output(i, x_ref, io_ref, wob_ref, kv_ref, phiq_ref)
                pl.when(block == 1)(out_copy(i).start)

    for i in range(S // TB2):
        out_copy(i).wait()


@functools.partial(jax.jit, static_argnames=("A_seg_len",))
def pallas_interleave_layers__memory_aug_recurrent_mem_tr__linear_kernel_hedgehog__prompt_kernel(
    A_x: jax.Array,
    A_mem0: jax.Array,
    A_Wq: jax.Array,
    A_Wk: jax.Array,
    A_Wv: jax.Array,
    A_Wo: jax.Array,
    A_seg_len: int,
    B_x: jax.Array,
    B_wqkv: jax.Array,
    B_w_phi: jax.Array,
    B_wo: jax.Array,
):
    del B_x
    assert A_x.shape == (1, S, D) and A_mem0.shape == (1, M, D) and A_seg_len == SEG
    assert A_Wq.shape == (D, H, DH) and B_w_phi.shape == (H, F, F)

    def head_major(w):
        return jnp.transpose(w, (1, 2, 0)).reshape(NP, PW, D)

    hbm = pl.BlockSpec(memory_space=pl.ANY)
    vmem = pl.BlockSpec(memory_space=pltpu.VMEM)
    out = pl.pallas_call(
        _kernel,
        out_shape=jax.ShapeDtypeStruct((S, D), bf16),
        in_specs=[hbm, hbm, vmem, hbm, hbm, hbm, hbm, hbm, vmem, hbm],
        out_specs=hbm,
        scratch_shapes=[
            pltpu.VMEM((S, D), f32),
            pltpu.VMEM((L, D), f32),
            pltpu.VMEM((S, D), bf16),
            pltpu.VMEM((NP, D // 2, 3 * PW), u32),
            pltpu.VMEM((NP, PW // 2, D), u32),
            pltpu.VMEM((NP, NSEG * AHEAD, 2 * PW), f32),
            pltpu.VMEM((2 * L + 64, 128), f32),
            pltpu.VMEM((NG, 3 * GW // 2, D), u32),
            pltpu.VMEM((D // 2, D), u32),
            pltpu.VMEM((NP, PF + 8, 2 * PF), f32),
            pltpu.VMEM((S // SUB, NP, PF, SUB), u32),
            pltpu.VMEM((S, D), bf16),
            pltpu.VMEM((NSEG, AHEAD, D), bf16),
            pltpu.VMEM((NSEG * AHEAD, D), bf16),
            pltpu.VMEM((NP, 4, PW, D), bf16),
            pltpu.VMEM((D, 3 * D), bf16),
            pltpu.VMEM((D, D), bf16),
            pltpu.SemaphoreType.DMA((NP, 4)),
            pltpu.SemaphoreType.DMA((5,)),
            pltpu.SemaphoreType.DMA((S // TB2,)),
        ],
        compiler_params=pltpu.CompilerParams(vmem_limit_bytes=120 * 1024 * 1024, flags=FLAGS),
    )(
        A_x.reshape(S, D),
        A_x.reshape(NSEG, SEG // AHEAD, AHEAD, D),
        A_mem0.reshape(M, D),
        head_major(A_Wq),
        head_major(A_Wk),
        head_major(A_Wv),
        A_Wo.reshape(NP, PW, D),
        B_wqkv,
        jnp.transpose(B_w_phi, (1, 2, 0)),
        B_wo,
    )
    return out.reshape(1, S, D)
```

```python
import functools

import jax
import jax.numpy as jnp
import jax.experimental.pallas as pl
import jax.experimental.pallas.tpu as pltpu

f32, bf16, u32, i32 = jnp.float32, jnp.bfloat16, jnp.uint32, jnp.int32

S, D = 2048, 640
H, DH = 32, 192
M, SEG = 8, 32
L = M + SEG
NSEG = S // SEG
NP = H // 2
PW = 2 * DH
LOG2E = 1.4426950408889634
SCALE = DH ** -0.5 * LOG2E
MASKED = -1e9 * LOG2E

AHEAD = 8
HEAD = SEG - AHEAD
UNROLL = 2
ORDER = ("qvqqvvkskookooopx", "qqvvqvskokokooopx")
LAGS = ("q0 k0 v1 s1 x1 p3 o6", "q0 k0 v1 s1 x1 p3 o5")
ON_VPU = ("1" * NP, "1" * NP)
PREFETCH, LATE = 4, 4
X_FIRST = 2 * UNROLL

F = D // H
PF = 2 * F
NG, GP = 4, 4
GW = PF * GP
TB, TB2, SUB = 512, 512, 128
FLAGS = None
BLAG = 2
MC, NC = 128, 384


def _nn(a, b):
    return jax.lax.dot_general(a, b, (((1,), (0,)), ((), ())), preferred_element_type=f32)


def _nt(a, b):
    return jax.lax.dot_general(a, b, (((1,), (1,)), ((), ())), preferred_element_type=f32)


def _tn(a, b):
    return jax.lax.dot_general(a, b, (((0,), (0,)), ((), ())), preferred_element_type=f32)


def _unpack(w):
    return pltpu.bitcast(w, bf16)


def _pack(w):
    return pltpu.bitcast(w.astype(bf16), u32)


def _iota(shape, dim):
    return jax.lax.broadcasted_iota(i32, shape, dim)


def _onehot(cond):
    return jnp.where(cond, 1.0, 0.0).astype(bf16)


def _rows(i, n):
    return pl.ds(pl.multiple_of(i * n, n), n)


def _recip(x):
    r = pl.reciprocal(x, approx=True)
    return r * (2.0 - x * r)


def _layernorm(x):
    xc = x - jnp.mean(x, axis=1, keepdims=True)
    var = jnp.mean(xc * xc, axis=1, keepdims=True)
    return xc * jax.lax.rsqrt(var + 1e-5)


def _store_caps(cap_ref):
    def position(i):
        return jnp.where(i < HEAD, i + M, jnp.where(i < HEAD + M, i - HEAD, i))

    query = position(_iota((L, 128), 0))
    for n in range(2):
        key = _iota((L, 128), 1) - n * L
        cap = jnp.where((query < M) | (query >= position(key)), jnp.inf, MASKED)
        cap_ref[n * L:(n + 1) * L] = jnp.where((key >= 0) & (key < L), cap, -jnp.inf)
    r = _iota((64, 128), 0)
    cap_ref[2 * L:2 * L + 64] = jnp.where((r & 7) >= (r >> 3), jnp.inf, MASKED)


def _a_segment(layer, s, mem, tok, wqkv_ref, wo_ref, pre_ref, cap_ref):
    lo, lo8 = _iota((L, 128), 1) < 64, _iota((8, 128), 1) < 64
    h = jnp.concatenate([tok[0:HEAD], mem, tok[HEAD:SEG]], axis=0)
    h_now = h[0:L - AHEAD].astype(bf16)
    q, k, v, prob, o_mxu, o_vpu, acc = {}, {}, {}, {}, {}, {}, {}

    def bands(top, bot):
        return jnp.concatenate(
            [jnp.concatenate(top, axis=1), jnp.concatenate(bot, axis=1),
             jnp.zeros((128 - 2 * L, 128 * len(top)), f32)], axis=0).astype(bf16)

    def lhs(t):
        return t.astype(bf16) if t.shape[0] % 16 == 0 else t

    def first_mxu_row(p):
        return 8 * int(ON_VPU[layer][p])

    def project(j, p, n):
        cols = slice(j * PW + n * 128, j * PW + (n + 1) * 128)
        w = _unpack(wqkv_ref[p, :, cols])
        if layer == 0 and j < 2:
            r = jnp.concatenate([_nn(h_now, w), pre_ref[p, _rows(s, AHEAD), cols]], axis=0)
        else:
            r = _nn(h, w)
        (q, k, v)[j][p, n] = r

    def scores(p):
        r0 = first_mxu_row(p)
        both = _nt(lhs(q[p, 1][r0:L]),
                   bands([jnp.where(lo, k[p, 1], 0.0)], [jnp.where(lo, 0.0, k[p, 1])]))
        rest = _nt(lhs(jnp.concatenate([q[p, 0][r0:L], q[p, 2][r0:L]], axis=0)),
                   bands([k[p, 0]], [k[p, 2]]))
        e = []
        for n in range(2):
            t = (both + rest[n * (L - r0):(n + 1) * (L - r0)]) * SCALE
            t = jnp.minimum(t, cap_ref[n * L + r0:(n + 1) * L])
            e.append(jnp.exp2(t - jnp.max(t, axis=1, keepdims=True)))
        total = [jnp.sum(t, axis=1, keepdims=True) for t in e]
        prob[p] = (e[0] + e[1], _recip(jnp.where(lo[r0:L], total[0], total[1])))

    def mix(p):
        e, inv = prob[p]
        o = _nn(lhs(e), bands([jnp.where(lo, v[p, n], 0.0) for n in range(3)],
                              [jnp.where(lo, 0.0, v[p, n]) for n in range(3)]))
        o_mxu[p] = o * jnp.concatenate([inv] * 3, axis=1)

    def attend_on_vpu(p):
        o_vpu[p] = []
        if not first_mxu_row(p):
            return
        q0, q1, q2 = (q[p, n][0:8] * SCALE for n in range(3))
        q1a, q1b = jnp.where(lo8, q1, 0.0), jnp.where(lo8, 0.0, q1)
        keys = list(range(HEAD, HEAD + M)) + list(range(8))

        def row(t, j):
            return [jnp.broadcast_to(t[p, n][j:j + 1], (8, 128)) for n in range(3)]

        sc = {}
        for j in keys:
            k0, k1, k2 = row(k, j)
            t = jnp.where(lo8, jnp.sum(q0 * k0 + q1a * k1, axis=1, keepdims=True),
                          jnp.sum(q1b * k1 + q2 * k2, axis=1, keepdims=True))
            if 0 < j < 8:
                t = jnp.minimum(t, cap_ref[2 * L + 8 * j:2 * L + 8 * j + 8])
            sc[j] = t
        top = functools.reduce(jnp.maximum, sc.values())
        o = None
        for j in keys:
            e = jnp.exp2(sc[j] - top)
            t = [e * x for x in row(v, j)] + [e]
            o = t if o is None else [x + y for x, y in zip(o, t)]
        inv = _recip(o[3])
        o_vpu[p] = [jnp.concatenate([x * inv for x in o[0:3]], axis=1)]

    def output(p, n):
        o = jnp.concatenate(o_vpu[p] + [o_mxu[p]], axis=0)
        o = jnp.concatenate([o[HEAD:HEAD + M], o[0:HEAD], o[HEAD + M:L]], axis=0)
        r = _nn(o, _unpack(wo_ref[p, :, n * 128:(n + 1) * 128]))
        acc[n] = acc[n] + r if n in acc else r

    stages = dict(q=functools.partial(project, 0), k=functools.partial(project, 1),
                  v=functools.partial(project, 2), o=output,
                  s=scores, p=mix, x=attend_on_vpu)
    lag = {w[0]: int(w[1:]) for w in LAGS[layer].split()}
    for t in range(NP + max(lag.values())):
        tile = dict(q=0, k=0, v=0, o=0)
        for name in ORDER[layer]:
            args = ()
            if name in tile:
                args = (tile[name],)
                tile[name] += 1
            if 0 <= t - lag[name] < NP:
                stages[name](t - lag[name], *args)
    out = jnp.concatenate([acc[n] for n in range(D // 128)], axis=1)
    return out[0:M], out[M:L]


def _store_ln(i, x_ref, ln_ref):
    rows = _rows(i, UNROLL * SEG)
    ln_ref[rows, :] = _layernorm(x_ref[rows, :]).astype(bf16)


def _a_steps(layer, i, read_x, x_ref, h_ref, ln_ref, *refs):
    _store_ln(jnp.maximum(i - 1, 0), x_ref, ln_ref)
    mem, tok = h_ref[0:M, :], h_ref[M:L, :]
    for u in range(UNROLL):
        s = i * UNROLL + u
        tok_next = _layernorm(read_x(jnp.minimum(s + 1, NSEG - 1)))
        mem, out = _a_segment(layer, s, mem, tok, *refs)
        x_ref[_rows(s, SEG), :] = read_x(s) + out
        tok = tok_next
    h_ref[0:M, :] = mem
    h_ref[M:L, :] = tok


def _over_features(op, rows):
    t = functools.reduce(op, rows)
    t = op(t, pltpu.roll(t, 4, 0))
    return op(t, pltpu.roll(t, 2, 0))


def _features(p):
    rows = [p[r:r + 8] * LOG2E for r in range(0, PF, 8)]
    hi, lo = _over_features(jnp.maximum, rows), _over_features(jnp.minimum, rows)
    out = []
    for e in ([jnp.exp2(r - hi) for r in rows], [jnp.exp2(lo - r) for r in rows]):
        inv = _recip(_over_features(jnp.add, e))
        out += [t * inv for t in e]
    return jnp.concatenate(out, axis=0)


def _b_accumulate(i, ln_ref, wb_ref, kv_ref, z_ref, phiq_ref):
    ln = ln_ref[_rows(i, TB), :]
    blocks = [slice(t * SUB, (t + 1) * SUB) for t in range(TB // SUB)]
    kv = {}
    for g in range(NG + 1):
        if g < NG:
            r = _nt(_unpack(wb_ref[g]), ln)
            for n in range(GP):
                pair = g * GP + n
                k, v, q = (r[j * GW + n * PF:j * GW + (n + 1) * PF] for j in range(3))
                phi_k, phi_q = _features(k), _pack(_features(q))
                kv[pair] = (v, phi_k.astype(bf16))
                z_ref[pair] += functools.reduce(jnp.add, [phi_k[:, b] for b in blocks])
                for t, b in enumerate(blocks):
                    phiq_ref[i * len(blocks) + t, pair] = phi_q[:, b]
        for n in range((g - 1) * GP, g * GP) if g else ():
            kv_ref[n] += _nt(*kv.pop(n))


def _b_finish(kv_ref, z_ref):
    row, col = _iota((PF, 2 * PF), 0), _iota((PF, 2 * PF), 1)
    same_head = jnp.where(row >= F, 1, 0) == (col & 1)
    for n in range(NP):
        kv_ref[n] = jnp.where(same_head, kv_ref[n], 0.0)
        z_ref[n] = jnp.broadcast_to(jnp.sum(z_ref[n], axis=1, keepdims=True), (2 * PF, SUB))


def _b_output(i, x_ref, io_ref, wob_ref, kv_ref, z_ref, phiq_ref):
    o = {}
    nsub = TB2 // SUB
    upper = _iota((8, SUB), 0) < F % 8
    for t in range(nsub + BLAG):
        if t < nsub:
            rows = []
            for n in range(NP):
                phi_q = _unpack(phiq_ref[i * nsub + t, n])
                num = _nn(kv_ref[n], phi_q)
                den = phi_q.astype(f32) * z_ref[n]
                den = _over_features(jnp.add, [den[r:r + 8] for r in range(0, 2 * PF, 8)])
                inv = 1.0 / (den + 1e-6)
                a, b = (jnp.broadcast_to(inv[j:j + 1], inv.shape) for j in range(2))
                rows += [num[8 * j:8 * j + 8] * c
                         for j, c in enumerate((a, a, jnp.where(upper, a, b), b, b))]
            o[t] = jnp.concatenate(rows, axis=0).astype(bf16)
        if t >= BLAG:
            blk = i * nsub + t - BLAG
            x = x_ref[_rows(blk, SUB), :] + _tn(o.pop(t - BLAG), _unpack(wob_ref[...]))
            x_ref[_rows(blk, SUB), :] = x
            io_ref[_rows(blk, SUB), :] = x.astype(bf16)


def _prepare_b(wqkv_ref, wphi_ref, wo_ref, wb_ref, wob_ref):
    hk, ck = _iota((H, D), 0), _iota((H, D), 1)
    phi = functools.reduce(
        jnp.add, [_nn(wphi_ref[d], _onehot(ck == hk * F + d)) for d in range(F)])

    def decode(row):
        pair = sum(jnp.where(row >= n * PF, 1, 0) for n in range(1, GP))
        return (row - pair * PF) >> 1, 2 * pair + (row & 1)

    spread = _onehot(decode(_iota((GW, F), 0))[0] == _iota((GW, F), 1))
    phi_rows = _nn(spread, phi.astype(bf16))
    cw = 256
    col = _iota((GW, cw), 1) - decode(_iota((GW, cw), 0))[1] * F
    wv = _pack(wqkv_ref[:, 2 * D:3 * D].T)
    for g in range(NG):
        c0 = g * 128
        d = col + (c0 - g * GW)
        fold = jnp.where((d >= 0) & (d < F), phi_rows[:, c0:c0 + cw], 0.0).astype(bf16)
        half = GW // 2
        wb_ref[g, 0:half] = _pack(_nt(fold, wqkv_ref[:, D + c0:D + c0 + cw]))
        wb_ref[g, half:2 * half] = wv[g * half:(g + 1) * half]
        wb_ref[g, 2 * half:3 * half] = _pack(_nt(fold, wqkv_ref[:, c0:c0 + cw]))
    wob_ref[...] = _pack(wo_ref[...])


def _kernel(x_hbm, x_tiles_hbm, mem0_ref, wq_hbm, wk_hbm, wv_hbm, wo_hbm,
            bqkv_hbm, wphi_ref, bwo_hbm, out_hbm,
            x_ref, h_ref, ln_ref, wqkv_ref, wo_ref, pre_ref, cap_ref,
            wb_ref, wob_ref, kv_ref, z_ref, phiq_ref,
            io_ref, tail_in_ref, tail_ref, stage_ref, bqkv_ref, bwo_ref, w_sem, sem, out_sem):
    first, rest = pl.ds(0, X_FIRST * SEG), pl.ds(X_FIRST * SEG, S - X_FIRST * SEG)
    x_first = pltpu.make_async_copy(x_hbm.at[first], io_ref.at[first], sem.at[0])
    x_rest = pltpu.make_async_copy(x_hbm.at[rest], io_ref.at[rest], sem.at[1])
    tail_copy = pltpu.make_async_copy(
        x_tiles_hbm.at[:, SEG // AHEAD - 1], tail_in_ref, sem.at[2])
    bqkv_copy = pltpu.make_async_copy(bqkv_hbm, bqkv_ref, sem.at[3])
    bwo_copy = pltpu.make_async_copy(bwo_hbm, bwo_ref, sem.at[4])

    def w_copy(p, j):
        src = (wq_hbm, wk_hbm, wv_hbm, wo_hbm)[j]
        return pltpu.make_async_copy(src.at[p], stage_ref.at[p, j], w_sem.at[p, j])

    def install(w, p, j):
        if j >= 2:
            w = jnp.concatenate(
                [w[r + c:r + c + 64] for c in range(0, DH, 64) for r in (0, DH)], axis=0)
        if j < 3:
            wqkv_ref[p, :, j * PW:(j + 1) * PW] = _pack(w.T)
        else:
            wo_ref[p] = _pack(w)

    early, late = (0, 1), (2, 3)
    tail_copy.start()
    w_copy(0, 0).start()
    _store_caps(cap_ref)
    tail_copy.wait()
    w_copy(0, 1).start()
    for p in range(1, PREFETCH):
        for j in early:
            w_copy(p, j).start()
    tail_ref[...] = _layernorm(
        tail_in_ref[...].astype(f32).reshape(NSEG * AHEAD, D)).astype(bf16)

    def load_pair(p):
        for j in early:
            w_copy(p, j).wait()

        @pl.when(p >= LATE)
        def _():
            for j in late:
                w_copy(p - LATE, j).wait()

        @pl.when(p + PREFETCH < NP)
        def _():
            for j in early:
                w_copy(p + PREFETCH, j).start()

        @pl.when(p == LATE)
        def _():
            for copy in (bqkv_copy, bwo_copy, x_first):
                copy.start()

        for j in late:
            w_copy(p, j).start()
        due = p >= LATE
        for j in late:
            install(stage_ref[jnp.where(due, p - LATE, p), jnp.where(due, j, j - 2)],
                    jnp.where(due, p - LATE, p - LATE + NP), j)
        for j in early:
            for r in range(0, NSEG * AHEAD, MC):
                for c in range(0, PW, NC):
                    pre_ref[p, r:r + MC, j * PW + c:j * PW + c + NC] = _nt(
                        tail_ref[r:r + MC], stage_ref[p, j, c:c + NC])
            install(stage_ref[p, j], p, j)

    with jax.named_scope("load"):
        pl.loop(0, NP)(load_pair)
    with jax.named_scope("bprep"):
        bqkv_copy.wait()
        bwo_copy.wait()
        _prepare_b(bqkv_ref, wphi_ref, bwo_ref, wb_ref, wob_ref)

        @pl.loop(NP - LATE, NP)
        def _(p):
            for j in late:
                w_copy(p, j).wait()
                install(stage_ref[p, j], p, j)
        x_first.wait()
        x_rest.start()
        x_ref[0:UNROLL * SEG, :] = io_ref[0:UNROLL * SEG, :].astype(f32)

    def out_copy(i):
        rows = _rows(i, TB2)
        return pltpu.make_async_copy(io_ref.at[rows], out_hbm.at[rows], out_sem.at[i])

    def layer_a(layer):
        def read_x(s):
            return (x_ref if layer else io_ref)[_rows(s, SEG), :].astype(f32)

        h_ref[0:M, :] = mem0_ref[...].astype(f32)
        h_ref[M:L, :] = _layernorm(x_ref[0:SEG, :])

        @pl.loop(0, NSEG // UNROLL)
        def _(i):
            if layer == 0:
                pl.when(i == 1)(x_rest.wait)
            _a_steps(layer, i, read_x, x_ref, h_ref, ln_ref, wqkv_ref, wo_ref, pre_ref, cap_ref)

    @pl.loop(0, 2)
    def _(block):
        with jax.named_scope("A"):
            for layer in range(2):
                pl.when(block == layer)(functools.partial(layer_a, layer))
        _store_ln(NSEG // UNROLL - 1, x_ref, ln_ref)
        kv_ref[...] = jnp.zeros(kv_ref.shape, f32)
        z_ref[...] = jnp.zeros(z_ref.shape, f32)
        with jax.named_scope("B1"):
            pl.loop(0, S // TB)(
                lambda i: _b_accumulate(i, ln_ref, wb_ref, kv_ref, z_ref, phiq_ref))
        _b_finish(kv_ref, z_ref)
        with jax.named_scope("B2"):
            @pl.loop(0, S // TB2)
            def _(i):
                _b_output(i, x_ref, io_ref, wob_ref, kv_ref, z_ref, phiq_ref)
                pl.when(block == 1)(out_copy(i).start)

    for i in range(S // TB2):
        out_copy(i).wait()


@functools.partial(jax.jit, static_argnames=("A_seg_len",))
def pallas_interleave_layers__memory_aug_recurrent_mem_tr__linear_kernel_hedgehog__prompt_kernel(
    A_x: jax.Array,
    A_mem0: jax.Array,
    A_Wq: jax.Array,
    A_Wk: jax.Array,
    A_Wv: jax.Array,
    A_Wo: jax.Array,
    A_seg_len: int,
    B_x: jax.Array,
    B_wqkv: jax.Array,
    B_w_phi: jax.Array,
    B_wo: jax.Array,
):
    del B_x
    assert A_x.shape == (1, S, D) and A_mem0.shape == (1, M, D) and A_seg_len == SEG
    assert A_Wq.shape == (D, H, DH) and B_w_phi.shape == (H, F, F)

    def head_major(w):
        return jnp.transpose(w, (1, 2, 0)).reshape(NP, PW, D)

    hbm = pl.BlockSpec(memory_space=pl.ANY)
    vmem = pl.BlockSpec(memory_space=pltpu.VMEM)
    out = pl.pallas_call(
        _kernel,
        out_shape=jax.ShapeDtypeStruct((S, D), bf16),
        in_specs=[hbm, hbm, vmem, hbm, hbm, hbm, hbm, hbm, vmem, hbm],
        out_specs=hbm,
        scratch_shapes=[
            pltpu.VMEM((S, D), f32),
            pltpu.VMEM((L, D), f32),
            pltpu.VMEM((S, D), bf16),
            pltpu.VMEM((NP, D // 2, 3 * PW), u32),
            pltpu.VMEM((NP, PW // 2, D), u32),
            pltpu.VMEM((NP, NSEG * AHEAD, 2 * PW), f32),
            pltpu.VMEM((2 * L + 64, 128), f32),
            pltpu.VMEM((NG, 3 * GW // 2, D), u32),
            pltpu.VMEM((D // 2, D), u32),
            pltpu.VMEM((NP, PF, 2 * PF), f32),
            pltpu.VMEM((NP, 2 * PF, SUB), f32),
            pltpu.VMEM((S // SUB, NP, PF, SUB), u32),
            pltpu.VMEM((S, D), bf16),
            pltpu.VMEM((NSEG, AHEAD, D), bf16),
            pltpu.VMEM((NSEG * AHEAD, D), bf16),
            pltpu.VMEM((NP, 4, PW, D), bf16),
            pltpu.VMEM((D, 3 * D), bf16),
            pltpu.VMEM((D, D), bf16),
            pltpu.SemaphoreType.DMA((NP, 4)),
            pltpu.SemaphoreType.DMA((5,)),
            pltpu.SemaphoreType.DMA((S // TB2,)),
        ],
        compiler_params=pltpu.CompilerParams(vmem_limit_bytes=120 * 1024 * 1024, flags=FLAGS),
    )(
        A_x.reshape(S, D),
        A_x.reshape(NSEG, SEG // AHEAD, AHEAD, D),
        A_mem0.reshape(M, D),
        head_major(A_Wq),
        head_major(A_Wk),
        head_major(A_Wv),
        A_Wo.reshape(NP, PW, D),
        B_wqkv,
        jnp.transpose(B_w_phi, (1, 2, 0)),
        B_wo,
    )
    return out.reshape(1, S, D)
```

```python
import functools

import jax
import jax.numpy as jnp
import jax.experimental.pallas as pl
import jax.experimental.pallas.tpu as pltpu

f32, bf16, u32, i32 = jnp.float32, jnp.bfloat16, jnp.uint32, jnp.int32

S, D = 2048, 640
H, DH = 32, 192
M, SEG = 8, 32
L = M + SEG
NSEG = S // SEG
NP = H // 2
PW = 2 * DH
LOG2E = 1.4426950408889634
SCALE = DH ** -0.5 * LOG2E
MASKED = -1e9 * LOG2E

AHEAD = 8
HEAD = SEG - AHEAD
UNROLL = 2
ORDER = ("qvqqvvkskookooopx", "qqvvqvskokokooopx")
LAGS = ("q0 k0 v1 s1 x1 p3 o6", "q0 k0 v1 s1 x1 p3 o5")
ON_VPU = ("1" * NP, "1" * NP)
PREFETCH, LATE = 4, 4
X_FIRST = 2 * UNROLL

F = D // H
PF = 2 * F
NG, GP = 4, 4
GW = PF * GP
TB, TB2, SUB = 512, 512, 128
FLAGS = None
BLAG = 2
MC, NC = 128, 384


def _nn(a, b):
    return jax.lax.dot_general(a, b, (((1,), (0,)), ((), ())), preferred_element_type=f32)


def _nt(a, b):
    return jax.lax.dot_general(a, b, (((1,), (1,)), ((), ())), preferred_element_type=f32)


def _tn(a, b):
    return jax.lax.dot_general(a, b, (((0,), (0,)), ((), ())), preferred_element_type=f32)


def _unpack(w):
    return pltpu.bitcast(w, bf16)


def _pack(w):
    return pltpu.bitcast(w.astype(bf16), u32)


def _iota(shape, dim):
    return jax.lax.broadcasted_iota(i32, shape, dim)


def _onehot(cond):
    return jnp.where(cond, 1.0, 0.0).astype(bf16)


def _rows(i, n):
    return pl.ds(pl.multiple_of(i * n, n), n)


def _recip(x):
    r = pl.reciprocal(x, approx=True)
    return r * (2.0 - x * r)


def _layernorm(x):
    xc = x - jnp.mean(x, axis=1, keepdims=True)
    var = jnp.mean(xc * xc, axis=1, keepdims=True)
    return xc * jax.lax.rsqrt(var + 1e-5)


def _store_caps(cap_ref):
    def position(i):
        return jnp.where(i < HEAD, i + M, jnp.where(i < HEAD + M, i - HEAD, i))

    query = position(_iota((L, 128), 0))
    for n in range(2):
        key = _iota((L, 128), 1) - n * L
        cap = jnp.where((query < M) | (query >= position(key)), jnp.inf, MASKED)
        cap_ref[n * L:(n + 1) * L] = jnp.where((key >= 0) & (key < L), cap, -jnp.inf)
    r = _iota((64, 128), 0)
    cap_ref[2 * L:2 * L + 64] = jnp.where((r & 7) >= (r >> 3), jnp.inf, MASKED)


def _a_segment(layer, s, mem, tok, wqkv_ref, wo_ref, pre_ref, cap_ref):
    lo, lo8 = _iota((L, 128), 1) < 64, _iota((8, 128), 1) < 64
    h = jnp.concatenate([tok[0:HEAD], mem, tok[HEAD:SEG]], axis=0)
    h_now = h[0:L - AHEAD].astype(bf16)
    q, k, v, prob, o_mxu, o_vpu, acc = {}, {}, {}, {}, {}, {}, {}

    def bands(top, bot):
        return jnp.concatenate(
            [jnp.concatenate(top, axis=1), jnp.concatenate(bot, axis=1),
             jnp.zeros((128 - 2 * L, 128 * len(top)), f32)], axis=0).astype(bf16)

    def lhs(t):
        return t.astype(bf16) if t.shape[0] % 16 == 0 else t

    def first_mxu_row(p):
        return 8 * int(ON_VPU[layer][p])

    def project(j, p, n):
        cols = slice(j * PW + n * 128, j * PW + (n + 1) * 128)
        w = _unpack(wqkv_ref[p, :, cols])
        if layer == 0 and j < 2:
            r = jnp.concatenate([_nn(h_now, w), pre_ref[p, _rows(s, AHEAD), cols]], axis=0)
        else:
            r = _nn(h, w)
        (q, k, v)[j][p, n] = r

    def scores(p):
        r0 = first_mxu_row(p)
        both = _nt(lhs(q[p, 1][r0:L]),
                   bands([jnp.where(lo, k[p, 1], 0.0)], [jnp.where(lo, 0.0, k[p, 1])]))
        rest = _nt(lhs(jnp.concatenate([q[p, 0][r0:L], q[p, 2][r0:L]], axis=0)),
                   bands([k[p, 0]], [k[p, 2]]))
        e = []
        for n in range(2):
            t = (both + rest[n * (L - r0):(n + 1) * (L - r0)]) * SCALE
            t = jnp.minimum(t, cap_ref[n * L + r0:(n + 1) * L])
            e.append(jnp.exp2(t - jnp.max(t, axis=1, keepdims=True)))
        total = [jnp.sum(t, axis=1, keepdims=True) for t in e]
        prob[p] = (e[0] + e[1], _recip(jnp.where(lo[r0:L], total[0], total[1])))

    def mix(p):
        e, inv = prob[p]
        o = _nn(lhs(e), bands([jnp.where(lo, v[p, n], 0.0) for n in range(3)],
                              [jnp.where(lo, 0.0, v[p, n]) for n in range(3)]))
        o_mxu[p] = o * jnp.concatenate([inv] * 3, axis=1)

    def attend_on_vpu(p):
        o_vpu[p] = []
        if not first_mxu_row(p):
            return
        q0, q1, q2 = (q[p, n][0:8] * SCALE for n in range(3))
        q1a, q1b = jnp.where(lo8, q1, 0.0), jnp.where(lo8, 0.0, q1)
        keys = list(range(HEAD, HEAD + M)) + list(range(8))

        def row(t, j):
            return [jnp.broadcast_to(t[p, n][j:j + 1], (8, 128)) for n in range(3)]

        sc = {}
        for j in keys:
            k0, k1, k2 = row(k, j)
            t = jnp.where(lo8, jnp.sum(q0 * k0 + q1a * k1, axis=1, keepdims=True),
                          jnp.sum(q1b * k1 + q2 * k2, axis=1, keepdims=True))
            if 0 < j < 8:
                t = jnp.minimum(t, cap_ref[2 * L + 8 * j:2 * L + 8 * j + 8])
            sc[j] = t
        top = functools.reduce(jnp.maximum, sc.values())
        o = None
        for j in keys:
            e = jnp.exp2(sc[j] - top)
            t = [e * x for x in row(v, j)] + [e]
            o = t if o is None else [x + y for x, y in zip(o, t)]
        inv = _recip(o[3])
        o_vpu[p] = [jnp.concatenate([x * inv for x in o[0:3]], axis=1)]

    def output(p, n):
        o = jnp.concatenate(o_vpu[p] + [o_mxu[p]], axis=0)
        o = jnp.concatenate([o[HEAD:HEAD + M], o[0:HEAD], o[HEAD + M:L]], axis=0)
        r = _nn(o, _unpack(wo_ref[p, :, n * 128:(n + 1) * 128]))
        acc[n] = acc[n] + r if n in acc else r

    stages = dict(q=functools.partial(project, 0), k=functools.partial(project, 1),
                  v=functools.partial(project, 2), o=output,
                  s=scores, p=mix, x=attend_on_vpu)
    lag = {w[0]: int(w[1:]) for w in LAGS[layer].split()}
    for t in range(NP + max(lag.values())):
        tile = dict(q=0, k=0, v=0, o=0)
        for name in ORDER[layer]:
            args = ()
            if name in tile:
                args = (tile[name],)
                tile[name] += 1
            if 0 <= t - lag[name] < NP:
                stages[name](t - lag[name], *args)
    out = jnp.concatenate([acc[n] for n in range(D // 128)], axis=1)
    return out[0:M], out[M:L]


def _store_ln(i, x_ref, ln_ref):
    rows = _rows(i, UNROLL * SEG)
    ln_ref[rows, :] = _layernorm(x_ref[rows, :]).astype(bf16)


def _a_steps(layer, i, read_x, x_ref, h_ref, ln_ref, *refs):
    _store_ln(jnp.maximum(i - 1, 0), x_ref, ln_ref)
    mem, tok = h_ref[0:M, :], h_ref[M:L, :]
    for u in range(UNROLL):
        s = i * UNROLL + u
        tok_next = _layernorm(read_x(jnp.minimum(s + 1, NSEG - 1)))
        mem, out = _a_segment(layer, s, mem, tok, *refs)
        x_ref[_rows(s, SEG), :] = read_x(s) + out
        tok = tok_next
    h_ref[0:M, :] = mem
    h_ref[M:L, :] = tok


def _over_features(op, rows):
    t = functools.reduce(op, rows)
    t = op(t, pltpu.roll(t, 4, 0))
    return op(t, pltpu.roll(t, 2, 0))


def _features(p):
    rows = [p[r:r + 8] * LOG2E for r in range(0, PF, 8)]
    hi, lo = _over_features(jnp.maximum, rows), _over_features(jnp.minimum, rows)
    out = []
    for e in ([jnp.exp2(r - hi) for r in rows], [jnp.exp2(lo - r) for r in rows]):
        inv = _recip(_over_features(jnp.add, e))
        out += [t * inv for t in e]
    return jnp.concatenate(out, axis=0)


def _b_accumulate(i, ln_ref, wb_ref, kv_ref, z_ref, phiq_ref):
    ln = ln_ref[_rows(i, TB), :]
    blocks = [slice(t * SUB, (t + 1) * SUB) for t in range(TB // SUB)]
    kv = {}
    for g in range(NG + 1):
        if g < NG:
            r = _nt(_unpack(wb_ref[g]), ln)
            for n in range(GP):
                pair = g * GP + n
                k, v, q = (r[j * GW + n * PF:j * GW + (n + 1) * PF] for j in range(3))
                phi_k, phi_q = _features(k), _pack(_features(q))
                kv[pair] = (v, phi_k.astype(bf16))
                z_ref[pair] += functools.reduce(jnp.add, [phi_k[:, b] for b in blocks])
                for t, b in enumerate(blocks):
                    phiq_ref[i * len(blocks) + t, pair] = phi_q[:, b]
        for n in range((g - 1) * GP, g * GP) if g else ():
            kv_ref[n] += _nt(*kv.pop(n))


def _b_finish(kv_ref, z_ref):
    row, col = _iota((PF, 2 * PF), 0), _iota((PF, 2 * PF), 1)
    same_head = jnp.where(row >= F, 1, 0) == (col & 1)
    for n in range(NP):
        kv_ref[n] = jnp.where(same_head, kv_ref[n], 0.0)
        z_ref[n] = jnp.broadcast_to(jnp.sum(z_ref[n], axis=1, keepdims=True), (2 * PF, SUB))


def _b_output(i, out_copy, x_ref, io_ref, wob_ref, kv_ref, z_ref, phiq_ref):
    o = {}
    nsub = TB2 // SUB
    upper = _iota((8, SUB), 0) < F % 8
    for t in range(nsub + BLAG):
        if t < nsub:
            rows = []
            for n in range(NP):
                phi_q = _unpack(phiq_ref[i * nsub + t, n])
                num = _nn(kv_ref[n], phi_q)
                den = phi_q.astype(f32) * z_ref[n]
                den = _over_features(jnp.add, [den[r:r + 8] for r in range(0, 2 * PF, 8)])
                inv = 1.0 / (den + 1e-6)
                a, b = (jnp.broadcast_to(inv[j:j + 1], inv.shape) for j in range(2))
                rows += [num[8 * j:8 * j + 8] * c
                         for j, c in enumerate((a, a, jnp.where(upper, a, b), b, b))]
            o[t] = jnp.concatenate(rows, axis=0).astype(bf16)
        if t >= BLAG:
            blk = i * nsub + t - BLAG
            x = x_ref[_rows(blk, SUB), :] + _tn(o.pop(t - BLAG), _unpack(wob_ref[...]))
            x_ref[_rows(blk, SUB), :] = x
            io_ref[_rows(blk, SUB), :] = x.astype(bf16)
            out_copy(blk).start()


def _decode(row):
    pair = sum(jnp.where(row >= n * PF, 1, 0) for n in range(1, GP))
    return (row - pair * PF) >> 1, 2 * pair + (row & 1)


def _spread_phi(wphi_ref, phi_ref):
    hk, ck = _iota((H, D), 0), _iota((H, D), 1)
    phi = functools.reduce(
        jnp.add, [_nn(wphi_ref[d], _onehot(ck == hk * F + d)) for d in range(F)])
    spread = _onehot(_decode(_iota((GW, F), 0))[0] == _iota((GW, F), 1))
    phi_ref[...] = _nn(spread, phi.astype(bf16))


def _fold_phi(g, wqkv_ref, phi_ref, wb_ref):
    cw = 256

    def cols(base):
        return pl.ds(pl.multiple_of(base + g * 128, 128), cw)

    d = _iota((GW, cw), 1) - _decode(_iota((GW, cw), 0))[1] * F + g * (128 - GW)
    fold = jnp.where((d >= 0) & (d < F), phi_ref[:, cols(0)], 0.0).astype(bf16)
    wb_ref[g, 0:GW // 2] = _pack(_nt(fold, wqkv_ref[:, cols(D)]))
    wb_ref[g, GW:3 * GW // 2] = _pack(_nt(fold, wqkv_ref[:, cols(0)]))


def _kernel(x_hbm, x_tiles_hbm, mem0_ref, wq_hbm, wk_hbm, wv_hbm, wo_hbm,
            bqkv_hbm, wphi_ref, bwo_hbm, out_hbm,
            x_ref, h_ref, ln_ref, wqkv_ref, wo_ref, pre_ref, cap_ref,
            wb_ref, wob_ref, kv_ref, z_ref, phiq_ref,
            io_ref, tail_in_ref, tail_ref, stage_ref, bqkv_ref, bwo_ref, phi_ref,
            w_sem, sem, out_sem):
    first, rest = pl.ds(0, X_FIRST * SEG), pl.ds(X_FIRST * SEG, S - X_FIRST * SEG)
    x_first = pltpu.make_async_copy(x_hbm.at[first], io_ref.at[first], sem.at[0])
    x_rest = pltpu.make_async_copy(x_hbm.at[rest], io_ref.at[rest], sem.at[1])
    tail_copy = pltpu.make_async_copy(
        x_tiles_hbm.at[:, SEG // AHEAD - 1], tail_in_ref, sem.at[2])
    bqkv_copy = pltpu.make_async_copy(bqkv_hbm, bqkv_ref, sem.at[3])
    bwo_copy = pltpu.make_async_copy(bwo_hbm, bwo_ref, sem.at[4])

    def w_copy(p, j):
        src = (wq_hbm, wk_hbm, wv_hbm, wo_hbm)[j]
        return pltpu.make_async_copy(src.at[p], stage_ref.at[p, j], w_sem.at[p, j])

    def install(w, p, j):
        if j >= 2:
            w = jnp.concatenate(
                [w[r + c:r + c + 64] for c in range(0, DH, 64) for r in (0, DH)], axis=0)
        if j < 3:
            wqkv_ref[p, :, j * PW:(j + 1) * PW] = _pack(w.T)
        else:
            wo_ref[p] = _pack(w)

    early, late = (0, 1), (2, 3)
    tail_copy.start()
    w_copy(0, 0).start()
    _store_caps(cap_ref)
    _spread_phi(wphi_ref, phi_ref)
    tail_copy.wait()
    w_copy(0, 1).start()
    for p in range(1, PREFETCH):
        for j in early:
            w_copy(p, j).start()
    tail_ref[...] = _layernorm(
        tail_in_ref[...].astype(f32).reshape(NSEG * AHEAD, D)).astype(bf16)

    def load_pair(p):
        for j in early:
            w_copy(p, j).wait()

        @pl.when(p >= LATE)
        def _():
            for j in late:
                w_copy(p - LATE, j).wait()

        @pl.when(p + PREFETCH < NP)
        def _():
            for j in early:
                w_copy(p + PREFETCH, j).start()

        @pl.when(p == LATE)
        def _():
            for copy in (bqkv_copy, bwo_copy, x_first):
                copy.start()

        for j in late:
            w_copy(p, j).start()
        due = p >= LATE
        for j in late:
            install(stage_ref[jnp.where(due, p - LATE, p), jnp.where(due, j, j - 2)],
                    jnp.where(due, p - LATE, p - LATE + NP), j)
        for j in early:
            for r in range(0, NSEG * AHEAD, MC):
                for c in range(0, PW, NC):
                    pre_ref[p, r:r + MC, j * PW + c:j * PW + c + NC] = _nt(
                        tail_ref[r:r + MC], stage_ref[p, j, c:c + NC])
            install(stage_ref[p, j], p, j)

    with jax.named_scope("load"):
        pl.loop(0, NP)(load_pair)
    with jax.named_scope("bprep"):
        bqkv_copy.wait()
        bwo_copy.wait()

        @pl.loop(0, NG)
        def _(g):
            p = NP - LATE + g
            for j in late:
                w_copy(p, j).wait()
            _fold_phi(g, bqkv_ref, phi_ref, wb_ref)
            for j in late:
                install(stage_ref[p, j], p, j)

        wv = _pack(bqkv_ref[:, 2 * D:3 * D].T)
        for g in range(NG):
            wb_ref[g, GW // 2:GW] = wv[g * GW // 2:(g + 1) * GW // 2]
        wob_ref[...] = _pack(bwo_ref[...])
        x_first.wait()
        x_rest.start()
        x_ref[0:UNROLL * SEG, :] = io_ref[0:UNROLL * SEG, :].astype(f32)

    def out_copy(i):
        rows = _rows(i, SUB)
        return pltpu.make_async_copy(io_ref.at[rows], out_hbm.at[rows], out_sem.at[i])

    def wait_for_output():
        for i in range(S // SUB):
            out_copy(i).wait()

    def layer_a(layer):
        def read_x(s):
            return (x_ref if layer else io_ref)[_rows(s, SEG), :].astype(f32)

        h_ref[0:M, :] = mem0_ref[...].astype(f32)
        h_ref[M:L, :] = _layernorm(x_ref[0:SEG, :])

        @pl.loop(0, NSEG // UNROLL)
        def _(i):
            if layer == 0:
                pl.when(i == 1)(x_rest.wait)
            _a_steps(layer, i, read_x, x_ref, h_ref, ln_ref, wqkv_ref, wo_ref, pre_ref, cap_ref)

        if layer == 1:
            wait_for_output()

    @pl.loop(0, 2)
    def _(block):
        with jax.named_scope("A"):
            for layer in range(2):
                pl.when(block == layer)(functools.partial(layer_a, layer))
        _store_ln(NSEG // UNROLL - 1, x_ref, ln_ref)
        kv_ref[...] = jnp.zeros(kv_ref.shape, f32)
        z_ref[...] = jnp.zeros(z_ref.shape, f32)
        with jax.named_scope("B1"):
            pl.loop(0, S // TB)(
                lambda i: _b_accumulate(i, ln_ref, wb_ref, kv_ref, z_ref, phiq_ref))
        _b_finish(kv_ref, z_ref)
        with jax.named_scope("B2"):
            pl.loop(0, S // TB2)(
                lambda i: _b_output(i, out_copy, x_ref, io_ref, wob_ref, kv_ref, z_ref, phiq_ref))

    wait_for_output()


@functools.partial(jax.jit, static_argnames=("A_seg_len",))
def pallas_interleave_layers__memory_aug_recurrent_mem_tr__linear_kernel_hedgehog__prompt_kernel(
    A_x: jax.Array,
    A_mem0: jax.Array,
    A_Wq: jax.Array,
    A_Wk: jax.Array,
    A_Wv: jax.Array,
    A_Wo: jax.Array,
    A_seg_len: int,
    B_x: jax.Array,
    B_wqkv: jax.Array,
    B_w_phi: jax.Array,
    B_wo: jax.Array,
):
    del B_x
    assert A_x.shape == (1, S, D) and A_mem0.shape == (1, M, D) and A_seg_len == SEG
    assert A_Wq.shape == (D, H, DH) and B_w_phi.shape == (H, F, F)

    def head_major(w):
        return jnp.transpose(w, (1, 2, 0)).reshape(NP, PW, D)

    hbm = pl.BlockSpec(memory_space=pl.ANY)
    vmem = pl.BlockSpec(memory_space=pltpu.VMEM)
    out = pl.pallas_call(
        _kernel,
        out_shape=jax.ShapeDtypeStruct((S, D), bf16),
        in_specs=[hbm, hbm, vmem, hbm, hbm, hbm, hbm, hbm, vmem, hbm],
        out_specs=hbm,
        scratch_shapes=[
            pltpu.VMEM((S, D), f32),
            pltpu.VMEM((L, D), f32),
            pltpu.VMEM((S, D), bf16),
            pltpu.VMEM((NP, D // 2, 3 * PW), u32),
            pltpu.VMEM((NP, PW // 2, D), u32),
            pltpu.VMEM((NP, NSEG * AHEAD, 2 * PW), f32),
            pltpu.VMEM((2 * L + 64, 128), f32),
            pltpu.VMEM((NG, 3 * GW // 2, D), u32),
            pltpu.VMEM((D // 2, D), u32),
            pltpu.VMEM((NP, PF, 2 * PF), f32),
            pltpu.VMEM((NP, 2 * PF, SUB), f32),
            pltpu.VMEM((S // SUB, NP, PF, SUB), u32),
            pltpu.VMEM((S, D), bf16),
            pltpu.VMEM((NSEG, AHEAD, D), bf16),
            pltpu.VMEM((NSEG * AHEAD, D), bf16),
            pltpu.VMEM((NP, 4, PW, D), bf16),
            pltpu.VMEM((D, 3 * D), bf16),
            pltpu.VMEM((D, D), bf16),
            pltpu.VMEM((GW, D), f32),
            pltpu.SemaphoreType.DMA((NP, 4)),
            pltpu.SemaphoreType.DMA((5,)),
            pltpu.SemaphoreType.DMA((S // SUB,)),
        ],
        compiler_params=pltpu.CompilerParams(vmem_limit_bytes=120 * 1024 * 1024, flags=FLAGS),
    )(
        A_x.reshape(S, D),
        A_x.reshape(NSEG, SEG // AHEAD, AHEAD, D),
        A_mem0.reshape(M, D),
        head_major(A_Wq),
        head_major(A_Wk),
        head_major(A_Wv),
        A_Wo.reshape(NP, PW, D),
        B_wqkv,
        jnp.transpose(B_w_phi, (1, 2, 0)),
        B_wo,
    )
    return out.reshape(1, S, D)
```

```python
import functools

import jax
import jax.numpy as jnp
import jax.experimental.pallas as pl
import jax.experimental.pallas.tpu as pltpu

f32, bf16, u32, i32 = jnp.float32, jnp.bfloat16, jnp.uint32, jnp.int32

S, D = 2048, 640
H, DH = 32, 192
M, SEG = 8, 32
L = M + SEG
NSEG = S // SEG
NP = H // 2
PW = 2 * DH
LOG2E = 1.4426950408889634
SCALE = DH ** -0.5 * LOG2E
MASKED = -1e9 * LOG2E

AHEAD = 8
HEAD = SEG - AHEAD
V = 8
UNROLL = 2
ORDER = ("qvqqvvkskookooopx", "qvvqqkvsokokooopx")
LAGS = ("q0 k0 v1 s1 x1 p3 o6", "q0 k0 v1 s1 x1 p3 o5")
PREFETCH, LATE = 4, 4
X_FIRST = 2 * UNROLL

F = D // H
PF = 2 * F
NG, GP = 4, 4
GW = PF * GP
TB, TB2, SUB = 512, 512, 128
BLAG = 2


def _nn(a, b):
    return jax.lax.dot_general(a, b, (((1,), (0,)), ((), ())), preferred_element_type=f32)


def _nt(a, b):
    return jax.lax.dot_general(a, b, (((1,), (1,)), ((), ())), preferred_element_type=f32)


def _tn(a, b):
    return jax.lax.dot_general(a, b, (((0,), (0,)), ((), ())), preferred_element_type=f32)


def _unpack(w):
    return pltpu.bitcast(w, bf16)


def _pack(w):
    return pltpu.bitcast(w.astype(bf16), u32)


def _iota(shape, dim):
    return jax.lax.broadcasted_iota(i32, shape, dim)


def _onehot(cond):
    return jnp.where(cond, 1.0, 0.0).astype(bf16)


def _rows(i, n):
    return pl.ds(pl.multiple_of(i * n, n), n)


def _recip(x):
    r = pl.reciprocal(x, approx=True)
    return r * (2.0 - x * r)


def _layernorm(x):
    xc = x - jnp.mean(x, axis=1, keepdims=True)
    var = jnp.mean(xc * xc, axis=1, keepdims=True)
    return xc * jax.lax.rsqrt(var + 1e-5)


def _store_caps(cap_ref):
    def position(i):
        return jnp.where(i < HEAD, i + M, jnp.where(i < HEAD + M, i - HEAD, i))

    query = position(_iota((L, 128), 0))
    for n in range(2):
        key = _iota((L, 128), 1) - n * L
        cap = jnp.where((query < M) | (query >= position(key)), jnp.inf, MASKED)
        cap_ref[n * L:(n + 1) * L] = jnp.where((key >= 0) & (key < L), cap, -jnp.inf)
    r = _iota((64, 128), 0)
    cap_ref[2 * L:2 * L + 64] = jnp.where((r & 7) >= (r >> 3), jnp.inf, MASKED)


def _a_segment(layer, s, mem, tok, wqkv_ref, wo_ref, pre_ref, cap_ref):
    lo, lo8 = _iota((L, 128), 1) < 64, _iota((8, 128), 1) < 64
    h = jnp.concatenate([tok[0:HEAD], mem, tok[HEAD:SEG]], axis=0)
    h_now = h[0:L - AHEAD].astype(bf16)
    q, k, v, prob, o_mxu, o_vpu, acc = {}, {}, {}, {}, {}, {}, {}

    def bands(top, bot):
        return jnp.concatenate(
            [jnp.concatenate(top, axis=1), jnp.concatenate(bot, axis=1),
             jnp.zeros((128 - 2 * L, 128 * len(top)), f32)], axis=0).astype(bf16)

    def project(j, p, n):
        cols = slice(j * PW + n * 128, j * PW + (n + 1) * 128)
        w = _unpack(wqkv_ref[p, :, cols])
        if layer == 0 and j < 2:
            r = jnp.concatenate([_nn(h_now, w), pre_ref[p, _rows(s, AHEAD), cols]], axis=0)
        else:
            r = _nn(h, w)
        (q, k, v)[j][p, n] = r

    def scores(p):
        both = _nt(q[p, 1][V:L].astype(bf16),
                   bands([jnp.where(lo, k[p, 1], 0.0)], [jnp.where(lo, 0.0, k[p, 1])]))
        rest = _nt(jnp.concatenate([q[p, 0][V:L], q[p, 2][V:L]], axis=0).astype(bf16),
                   bands([k[p, 0]], [k[p, 2]]))
        e = []
        for n in range(2):
            t = (both + rest[n * (L - V):(n + 1) * (L - V)]) * SCALE
            t = jnp.minimum(t, cap_ref[n * L + V:(n + 1) * L])
            e.append(jnp.exp2(t - jnp.max(t, axis=1, keepdims=True)))
        total = [jnp.sum(t, axis=1, keepdims=True) for t in e]
        prob[p] = (e[0] + e[1], _recip(jnp.where(lo[V:L], total[0], total[1])))

    def mix(p):
        e, inv = prob[p]
        o = _nn(e.astype(bf16), bands([jnp.where(lo, v[p, n], 0.0) for n in range(3)],
                                      [jnp.where(lo, 0.0, v[p, n]) for n in range(3)]))
        o_mxu[p] = o * jnp.concatenate([inv] * 3, axis=1)

    def attend_on_vpu(p):
        q0, q1, q2 = (q[p, n][0:8] * SCALE for n in range(3))
        q1a, q1b = jnp.where(lo8, q1, 0.0), jnp.where(lo8, 0.0, q1)
        keys = list(range(HEAD, HEAD + M)) + list(range(8))

        def row(t, j):
            block = [t[p, n][j // 8 * 8:j // 8 * 8 + 8] for n in range(3)]
            return [pltpu.roll(x, j % 8, 0) if j % 8 else x for x in block]

        sc = {}
        for j in keys:
            k0, k1, k2 = row(k, j)
            t = jnp.where(lo8, jnp.sum(q0 * k0 + q1a * k1, axis=1, keepdims=True),
                          jnp.sum(q1b * k1 + q2 * k2, axis=1, keepdims=True))
            if 0 < j < 8:
                t = jnp.minimum(t, cap_ref[2 * L + 8 * j:2 * L + 8 * j + 8])
            sc[j] = t
        top = functools.reduce(jnp.maximum, sc.values())
        o = None
        for j in keys:
            e = jnp.exp2(sc[j] - top)
            t = [e * x for x in row(v, j)] + [e]
            o = t if o is None else [x + y for x, y in zip(o, t)]
        inv = _recip(o[3])
        o_vpu[p] = jnp.concatenate([x * inv for x in o[0:3]], axis=1)

    def output(p, n):
        o = jnp.concatenate([o_vpu[p], o_mxu[p]], axis=0)
        o = jnp.concatenate([o[HEAD:HEAD + M], o[0:HEAD], o[HEAD + M:L]], axis=0)
        r = _nn(o, _unpack(wo_ref[p, :, n * 128:(n + 1) * 128]))
        acc[n] = acc[n] + r if n in acc else r

    stages = dict(q=functools.partial(project, 0), k=functools.partial(project, 1),
                  v=functools.partial(project, 2), o=output,
                  s=scores, p=mix, x=attend_on_vpu)
    lag = {w[0]: int(w[1:]) for w in LAGS[layer].split()}
    for t in range(NP + max(lag.values())):
        tile = dict(q=0, k=0, v=0, o=0)
        for name in ORDER[layer]:
            args = ()
            if name in tile:
                args = (tile[name],)
                tile[name] += 1
            if 0 <= t - lag[name] < NP:
                stages[name](t - lag[name], *args)
    out = jnp.concatenate([acc[n] for n in range(D // 128)], axis=1)
    return out[0:M], out[M:L]


def _store_ln(i, x_ref, ln_ref):
    rows = _rows(i, UNROLL * SEG)
    ln_ref[rows, :] = _layernorm(x_ref[rows, :]).astype(bf16)


def _a_steps(layer, i, read_x, x_ref, h_ref, ln_ref, *refs):
    _store_ln(jnp.maximum(i - 1, 0), x_ref, ln_ref)
    mem, tok = h_ref[0:M, :], h_ref[M:L, :]
    for u in range(UNROLL):
        s = i * UNROLL + u
        tok_next = _layernorm(read_x(jnp.minimum(s + 1, NSEG - 1)))
        mem, out = _a_segment(layer, s, mem, tok, *refs)
        x_ref[_rows(s, SEG), :] = read_x(s) + out
        tok = tok_next
    h_ref[0:M, :] = mem
    h_ref[M:L, :] = tok


def _over_features(op, rows):
    t = functools.reduce(op, rows)
    t = op(t, pltpu.roll(t, 4, 0))
    return op(t, pltpu.roll(t, 2, 0))


def _features(p):
    rows = [p[r:r + 8] * LOG2E for r in range(0, PF, 8)]
    hi, lo = _over_features(jnp.maximum, rows), _over_features(jnp.minimum, rows)
    out = []
    for e in ([jnp.exp2(r - hi) for r in rows], [jnp.exp2(lo - r) for r in rows]):
        inv = _recip(_over_features(jnp.add, e))
        out += [t * inv for t in e]
    return jnp.concatenate(out, axis=0)


def _b_accumulate(i, ln_ref, wb_ref, kv_ref, z_ref, phiq_ref):
    ln = ln_ref[_rows(i, TB), :]
    blocks = [slice(t * SUB, (t + 1) * SUB) for t in range(TB // SUB)]
    kv = {}
    for g in range(NG + 1):
        if g < NG:
            r = _nt(_unpack(wb_ref[g]), ln)
            for n in range(GP):
                pair = g * GP + n
                k, v, q = (r[j * GW + n * PF:j * GW + (n + 1) * PF] for j in range(3))
                phi_k, phi_q = _features(k), _pack(_features(q))
                kv[pair] = (v, phi_k.astype(bf16))
                z_ref[pair] += functools.reduce(jnp.add, [phi_k[:, b] for b in blocks])
                for t, b in enumerate(blocks):
                    phiq_ref[i * len(blocks) + t, pair] = phi_q[:, b]
        for n in range((g - 1) * GP, g * GP) if g else ():
            kv_ref[n] += _nt(*kv.pop(n))


def _b_finish(kv_ref, z_ref):
    row, col = _iota((PF, 2 * PF), 0), _iota((PF, 2 * PF), 1)
    same_head = jnp.where(row >= F, 1, 0) == (col & 1)
    for n in range(NP):
        kv_ref[n] = jnp.where(same_head, kv_ref[n], 0.0)
        z_ref[n] = jnp.broadcast_to(jnp.sum(z_ref[n], axis=1, keepdims=True), (2 * PF, SUB))


def _b_output(i, out_copy, x_ref, io_ref, wob_ref, kv_ref, z_ref, phiq_ref):
    o = {}
    nsub = TB2 // SUB
    upper = _iota((8, SUB), 0) < F % 8
    for t in range(nsub + BLAG):
        if t < nsub:
            rows = []
            for n in range(NP):
                phi_q = _unpack(phiq_ref[i * nsub + t, n])
                num = _nn(kv_ref[n], phi_q)
                den = phi_q.astype(f32) * z_ref[n]
                den = _over_features(jnp.add, [den[r:r + 8] for r in range(0, 2 * PF, 8)])
                inv = 1.0 / (den + 1e-6)
                a, b = (jnp.broadcast_to(inv[j:j + 1], inv.shape) for j in range(2))
                rows += [num[8 * j:8 * j + 8] * c
                         for j, c in enumerate((a, a, jnp.where(upper, a, b), b, b))]
            o[t] = jnp.concatenate(rows, axis=0).astype(bf16)
        if t >= BLAG:
            blk = i * nsub + t - BLAG
            x = x_ref[_rows(blk, SUB), :] + _tn(o.pop(t - BLAG), _unpack(wob_ref[...]))
            x_ref[_rows(blk, SUB), :] = x
            io_ref[_rows(blk, SUB), :] = x.astype(bf16)
            out_copy(blk).start()


def _decode(row):
    pair = sum(jnp.where(row >= n * PF, 1, 0) for n in range(1, GP))
    return (row - pair * PF) >> 1, 2 * pair + (row & 1)


def _spread_phi(wphi_ref, phi_ref):
    hk, ck = _iota((H, D), 0), _iota((H, D), 1)
    phi = functools.reduce(
        jnp.add, [_nn(wphi_ref[d], _onehot(ck == hk * F + d)) for d in range(F)])
    spread = _onehot(_decode(_iota((GW, F), 0))[0] == _iota((GW, F), 1))
    phi_ref[...] = _nn(spread, phi.astype(bf16))


def _fold_phi(g, wqkv_ref, phi_ref, wb_ref):
    cw = 256

    def cols(base):
        return pl.ds(pl.multiple_of(base + g * 128, 128), cw)

    d = _iota((GW, cw), 1) - _decode(_iota((GW, cw), 0))[1] * F + g * (128 - GW)
    fold = jnp.where((d >= 0) & (d < F), phi_ref[:, cols(0)], 0.0).astype(bf16)
    wb_ref[g, 0:GW // 2] = _pack(_nt(fold, wqkv_ref[:, cols(D)]))
    wb_ref[g, GW:3 * GW // 2] = _pack(_nt(fold, wqkv_ref[:, cols(0)]))


def _kernel(x_hbm, x_tiles_hbm, mem0_ref, wq_hbm, wk_hbm, wv_hbm, wo_hbm,
            bqkv_hbm, wphi_ref, bwo_hbm, out_hbm,
            x_ref, h_ref, ln_ref, wqkv_ref, wo_ref, pre_ref, cap_ref,
            wb_ref, wob_ref, kv_ref, z_ref, phiq_ref,
            io_ref, tail_in_ref, tail_ref, stage_ref, bqkv_ref, bwo_ref, phi_ref,
            w_sem, sem, out_sem):
    first, rest = pl.ds(0, X_FIRST * SEG), pl.ds(X_FIRST * SEG, S - X_FIRST * SEG)
    x_first = pltpu.make_async_copy(x_hbm.at[first], io_ref.at[first], sem.at[0])
    x_rest = pltpu.make_async_copy(x_hbm.at[rest], io_ref.at[rest], sem.at[1])
    tail_copy = pltpu.make_async_copy(
        x_tiles_hbm.at[:, SEG // AHEAD - 1], tail_in_ref, sem.at[2])
    bqkv_copy = pltpu.make_async_copy(bqkv_hbm, bqkv_ref, sem.at[3])
    bwo_copy = pltpu.make_async_copy(bwo_hbm, bwo_ref, sem.at[4])

    def w_copy(p, j):
        src = (wq_hbm, wk_hbm, wv_hbm, wo_hbm)[j]
        return pltpu.make_async_copy(src.at[p], stage_ref.at[p, j], w_sem.at[p, j])

    def install(w, p, j):
        if j >= 2:
            w = jnp.concatenate(
                [w[r + c:r + c + 64] for c in range(0, DH, 64) for r in (0, DH)], axis=0)
        if j < 3:
            wqkv_ref[p, :, j * PW:(j + 1) * PW] = _pack(w.T)
        else:
            wo_ref[p] = _pack(w)

    early, late = (0, 1), (2, 3)
    tail_copy.start()
    w_copy(0, 0).start()
    _store_caps(cap_ref)
    _spread_phi(wphi_ref, phi_ref)
    tail_copy.wait()
    w_copy(0, 1).start()
    for p in range(1, PREFETCH):
        for j in early:
            w_copy(p, j).start()
    tail_ref[...] = _layernorm(
        tail_in_ref[...].astype(f32).reshape(NSEG * AHEAD, D)).astype(bf16)

    def load_pair(p):
        for j in early:
            w_copy(p, j).wait()

        @pl.when(p >= LATE)
        def _():
            for j in late:
                w_copy(p - LATE, j).wait()

        @pl.when(p + PREFETCH < NP)
        def _():
            for j in early:
                w_copy(p + PREFETCH, j).start()

        @pl.when(p == LATE)
        def _():
            for copy in (bqkv_copy, bwo_copy, x_first):
                copy.start()

        for j in late:
            w_copy(p, j).start()
        for j in early:
            install(stage_ref[p, j], p, j)
        due = p >= LATE
        for j in late:
            install(stage_ref[jnp.where(due, p - LATE, p), jnp.where(due, j, j - 2)],
                    jnp.where(due, p - LATE, p - LATE + NP), j)
        for j in early:
            for r in range(0, NSEG * AHEAD, 128):
                pre_ref[p, r:r + 128, j * PW:(j + 1) * PW] = _nt(
                    tail_ref[r:r + 128], stage_ref[p, j])

    pl.loop(0, NP)(load_pair)
    bqkv_copy.wait()
    bwo_copy.wait()

    @pl.loop(0, NG)
    def _(g):
        p = NP - LATE + g
        for j in late:
            w_copy(p, j).wait()
        _fold_phi(g, bqkv_ref, phi_ref, wb_ref)
        for j in late:
            install(stage_ref[p, j], p, j)

    wv = _pack(bqkv_ref[:, 2 * D:3 * D].T)
    for g in range(NG):
        wb_ref[g, GW // 2:GW] = wv[g * GW // 2:(g + 1) * GW // 2]
    wob_ref[...] = _pack(bwo_ref[...])
    x_first.wait()
    x_rest.start()
    x_ref[0:UNROLL * SEG, :] = io_ref[0:UNROLL * SEG, :].astype(f32)

    def out_copy(i):
        rows = _rows(i, SUB)
        return pltpu.make_async_copy(io_ref.at[rows], out_hbm.at[rows], out_sem.at[i])

    def wait_for_output():
        for i in range(S // SUB):
            out_copy(i).wait()

    def layer_a(layer):
        def read_x(s):
            return (x_ref if layer else io_ref)[_rows(s, SEG), :].astype(f32)

        h_ref[0:M, :] = mem0_ref[...].astype(f32)
        h_ref[M:L, :] = _layernorm(x_ref[0:SEG, :])

        @pl.loop(0, NSEG // UNROLL)
        def _(i):
            if layer == 0:
                pl.when(i == 1)(x_rest.wait)
            _a_steps(layer, i, read_x, x_ref, h_ref, ln_ref, wqkv_ref, wo_ref, pre_ref, cap_ref)

        if layer == 1:
            wait_for_output()

    @pl.loop(0, 2)
    def _(block):
        for layer in range(2):
            pl.when(block == layer)(functools.partial(layer_a, layer))
        _store_ln(NSEG // UNROLL - 1, x_ref, ln_ref)
        kv_ref[...] = jnp.zeros(kv_ref.shape, f32)
        z_ref[...] = jnp.zeros(z_ref.shape, f32)
        pl.loop(0, S // TB)(
            lambda i: _b_accumulate(i, ln_ref, wb_ref, kv_ref, z_ref, phiq_ref))
        _b_finish(kv_ref, z_ref)
        pl.loop(0, S // TB2)(
            lambda i: _b_output(i, out_copy, x_ref, io_ref, wob_ref, kv_ref, z_ref, phiq_ref))

    wait_for_output()


@functools.partial(jax.jit, static_argnames=("A_seg_len",))
def pallas_interleave_layers__memory_aug_recurrent_mem_tr__linear_kernel_hedgehog__prompt_kernel(
    A_x: jax.Array,
    A_mem0: jax.Array,
    A_Wq: jax.Array,
    A_Wk: jax.Array,
    A_Wv: jax.Array,
    A_Wo: jax.Array,
    A_seg_len: int,
    B_x: jax.Array,
    B_wqkv: jax.Array,
    B_w_phi: jax.Array,
    B_wo: jax.Array,
):
    del B_x
    assert A_x.shape == (1, S, D) and A_mem0.shape == (1, M, D) and A_seg_len == SEG
    assert A_Wq.shape == (D, H, DH) and B_w_phi.shape == (H, F, F)

    def head_major(w):
        return jnp.transpose(w, (1, 2, 0)).reshape(NP, PW, D)

    hbm = pl.BlockSpec(memory_space=pl.ANY)
    vmem = pl.BlockSpec(memory_space=pltpu.VMEM)
    out = pl.pallas_call(
        _kernel,
        out_shape=jax.ShapeDtypeStruct((S, D), bf16),
        in_specs=[hbm, hbm, vmem, hbm, hbm, hbm, hbm, hbm, vmem, hbm],
        out_specs=hbm,
        scratch_shapes=[
            pltpu.VMEM((S, D), f32),
            pltpu.VMEM((L, D), f32),
            pltpu.VMEM((S, D), bf16),
            pltpu.VMEM((NP, D // 2, 3 * PW), u32),
            pltpu.VMEM((NP, PW // 2, D), u32),
            pltpu.VMEM((NP, NSEG * AHEAD, 2 * PW), f32),
            pltpu.VMEM((2 * L + 64, 128), f32),
            pltpu.VMEM((NG, 3 * GW // 2, D), u32),
            pltpu.VMEM((D // 2, D), u32),
            pltpu.VMEM((NP, PF, 2 * PF), f32),
            pltpu.VMEM((NP, 2 * PF, SUB), f32),
            pltpu.VMEM((S // SUB, NP, PF, SUB), u32),
            pltpu.VMEM((S, D), bf16),
            pltpu.VMEM((NSEG, AHEAD, D), bf16),
            pltpu.VMEM((NSEG * AHEAD, D), bf16),
            pltpu.VMEM((NP, 4, PW, D), bf16),
            pltpu.VMEM((D, 3 * D), bf16),
            pltpu.VMEM((D, D), bf16),
            pltpu.VMEM((GW, D), f32),
            pltpu.SemaphoreType.DMA((NP, 4)),
            pltpu.SemaphoreType.DMA((5,)),
            pltpu.SemaphoreType.DMA((S // SUB,)),
        ],
        compiler_params=pltpu.CompilerParams(vmem_limit_bytes=120 * 1024 * 1024),
    )(
        A_x.reshape(S, D),
        A_x.reshape(NSEG, SEG // AHEAD, AHEAD, D),
        A_mem0.reshape(M, D),
        head_major(A_Wq),
        head_major(A_Wk),
        head_major(A_Wv),
        A_Wo.reshape(NP, PW, D),
        B_wqkv,
        jnp.transpose(B_w_phi, (1, 2, 0)),
        B_wo,
    )
    return out.reshape(1, S, D)
```

```python
import functools

import jax
import jax.numpy as jnp
import jax.experimental.pallas as pl
import jax.experimental.pallas.tpu as pltpu

f32, bf16, u32, i32 = jnp.float32, jnp.bfloat16, jnp.uint32, jnp.int32

S, D = 2048, 640
H, DH = 32, 192
M, SEG = 8, 32
L = M + SEG
NSEG = S // SEG
NP = H // 2
PW = 2 * DH
LOG2E = 1.4426950408889634
SCALE = DH ** -0.5 * LOG2E
MASKED = -1e9 * LOG2E

V = 8
UNROLL = 2
ORDER = ("qvqqvsvkkookooopx", "vqvqqkvsokokooopx")
LAGS = ("q0 k0 v1 s1 x1 p3 o6", "q0 k0 v1 s1 x1 p3 o5")
PREFETCH, LATE = 4, 4
X_FIRST = 2 * UNROLL

F = D // H
PF = 2 * F
NG, GP = 4, 4
GW = PF * GP
TB, TB2, SUB = 512, 512, 128
BLAG = 2


def _nn(a, b):
    return jax.lax.dot_general(a, b, (((1,), (0,)), ((), ())), preferred_element_type=f32)


def _nt(a, b):
    return jax.lax.dot_general(a, b, (((1,), (1,)), ((), ())), preferred_element_type=f32)


def _tn(a, b):
    return jax.lax.dot_general(a, b, (((0,), (0,)), ((), ())), preferred_element_type=f32)


def _unpack(w):
    return pltpu.bitcast(w, bf16)


def _pack(w):
    return pltpu.bitcast(w.astype(bf16), u32)


def _iota(shape, dim):
    return jax.lax.broadcasted_iota(i32, shape, dim)


def _onehot(cond):
    return jnp.where(cond, 1.0, 0.0).astype(bf16)


def _rows(i, n):
    return pl.ds(pl.multiple_of(i * n, n), n)


def _recip(x):
    r = pl.reciprocal(x, approx=True)
    return r * (2.0 - x * r)


def _layernorm(x):
    xc = x - jnp.mean(x, axis=1, keepdims=True)
    var = jnp.mean(xc * xc, axis=1, keepdims=True)
    return xc * jax.lax.rsqrt(var + 1e-5)


def _store_caps(cap_ref):
    def position(i):
        return jnp.where(i < SEG, i + M, i - SEG)

    query = position(_iota((L, 128), 0))
    for n in range(2):
        key = _iota((L, 128), 1) - n * L
        cap = jnp.where((query < M) | (query >= position(key)), jnp.inf, MASKED)
        cap_ref[n * L:(n + 1) * L] = jnp.where((key >= 0) & (key < L), cap, -jnp.inf)
    r = _iota((64, 128), 0)
    cap_ref[2 * L:2 * L + 64] = jnp.where((r & 7) >= (r >> 3), jnp.inf, MASKED)


def _a_segment(layer, s, mem, tok, wqkv_ref, wo_ref, pre_ref, cap_ref):
    lo, lo8 = _iota((L, 128), 1) < 64, _iota((8, 128), 1) < 64
    h = jnp.concatenate([tok, mem], axis=0)
    h_rest = h[V:L].astype(bf16)
    q, k, v, prob, o_mxu, o_vpu, acc = {}, {}, {}, {}, {}, {}, {}

    def bands(top, bot):
        return jnp.concatenate(
            [jnp.concatenate(top, axis=1), jnp.concatenate(bot, axis=1),
             jnp.zeros((128 - 2 * L, 128 * len(top)), f32)], axis=0).astype(bf16)

    def project(j, p, n):
        cols = slice(j * PW + n * 128, j * PW + (n + 1) * 128)
        w = _unpack(wqkv_ref[p, :, cols])
        if layer == 0 and j < 2:
            r = jnp.concatenate([pre_ref[p, _rows(s, V), cols], _nn(h_rest, w)], axis=0)
        else:
            r = _nn(h, w)
        (q, k, v)[j][p, n] = r

    def scores(p):
        both = _nt(q[p, 1][V:L].astype(bf16),
                   bands([jnp.where(lo, k[p, 1], 0.0)], [jnp.where(lo, 0.0, k[p, 1])]))
        rest = _nt(jnp.concatenate([q[p, 0][V:L], q[p, 2][V:L]], axis=0).astype(bf16),
                   bands([k[p, 0]], [k[p, 2]]))
        e = []
        for n in range(2):
            t = (both + rest[n * (L - V):(n + 1) * (L - V)]) * SCALE
            t = jnp.minimum(t, cap_ref[n * L + V:(n + 1) * L])
            e.append(jnp.exp2(t - jnp.max(t, axis=1, keepdims=True)))
        total = [jnp.sum(t, axis=1, keepdims=True) for t in e]
        prob[p] = (e[0] + e[1], _recip(jnp.where(lo[V:L], total[0], total[1])))

    def mix(p):
        e, inv = prob[p]
        o = _nn(e.astype(bf16), bands([jnp.where(lo, v[p, n], 0.0) for n in range(3)],
                                      [jnp.where(lo, 0.0, v[p, n]) for n in range(3)]))
        o_mxu[p] = o * jnp.concatenate([inv] * 3, axis=1)

    def attend_on_vpu(p):
        q0, q1, q2 = (q[p, n][0:8] * SCALE for n in range(3))
        q1a, q1b = jnp.where(lo8, q1, 0.0), jnp.where(lo8, 0.0, q1)
        keys = list(range(SEG, L)) + list(range(V))

        def row(t, j):
            block = [t[p, n][j // 8 * 8:j // 8 * 8 + 8] for n in range(3)]
            return [pltpu.roll(x, j % 8, 0) if j % 8 else x for x in block]

        sc = {}
        for j in keys:
            k0, k1, k2 = row(k, j)
            t = jnp.where(lo8, jnp.sum(q0 * k0 + q1a * k1, axis=1, keepdims=True),
                          jnp.sum(q1b * k1 + q2 * k2, axis=1, keepdims=True))
            if 0 < j < 8:
                t = jnp.minimum(t, cap_ref[2 * L + 8 * j:2 * L + 8 * j + 8])
            sc[j] = t
        top = functools.reduce(jnp.maximum, sc.values())
        o = None
        for j in keys:
            e = jnp.exp2(sc[j] - top)
            t = [e * x for x in row(v, j)] + [e]
            o = t if o is None else [x + y for x, y in zip(o, t)]
        inv = _recip(o[3])
        o_vpu[p] = jnp.concatenate([x * inv for x in o[0:3]], axis=1)

    def output(p, n):
        o = jnp.concatenate([o_vpu[p], o_mxu[p]], axis=0)
        o = jnp.concatenate([o[SEG:L], o[0:SEG]], axis=0)
        r = _nn(o, _unpack(wo_ref[p, :, n * 128:(n + 1) * 128]))
        acc[n] = acc[n] + r if n in acc else r

    stages = dict(q=functools.partial(project, 0), k=functools.partial(project, 1),
                  v=functools.partial(project, 2), o=output,
                  s=scores, p=mix, x=attend_on_vpu)
    lag = {w[0]: int(w[1:]) for w in LAGS[layer].split()}
    for t in range(NP + max(lag.values())):
        tile = dict(q=0, k=0, v=0, o=0)
        for name in ORDER[layer]:
            args = ()
            if name in tile:
                args = (tile[name],)
                tile[name] += 1
            if 0 <= t - lag[name] < NP:
                stages[name](t - lag[name], *args)
    out = jnp.concatenate([acc[n] for n in range(D // 128)], axis=1)
    return out[0:M], out[M:L]


def _store_ln(i, x_ref, ln_ref):
    rows = _rows(i, UNROLL * SEG)
    ln_ref[rows, :] = _layernorm(x_ref[rows, :]).astype(bf16)


def _a_steps(layer, i, read_x, x_ref, h_ref, ln_ref, *refs):
    _store_ln(jnp.maximum(i - 1, 0), x_ref, ln_ref)
    mem, tok = h_ref[0:M, :], h_ref[M:L, :]
    for u in range(UNROLL):
        s = i * UNROLL + u
        tok_next = _layernorm(read_x(jnp.minimum(s + 1, NSEG - 1)))
        mem, out = _a_segment(layer, s, mem, tok, *refs)
        x_ref[_rows(s, SEG), :] = read_x(s) + out
        tok = tok_next
    h_ref[0:M, :] = mem
    h_ref[M:L, :] = tok


def _over_features(op, rows):
    t = functools.reduce(op, rows)
    t = op(t, pltpu.roll(t, 4, 0))
    return op(t, pltpu.roll(t, 2, 0))


def _features(p):
    rows = [p[r:r + 8] * LOG2E for r in range(0, PF, 8)]
    hi, lo = _over_features(jnp.maximum, rows), _over_features(jnp.minimum, rows)
    out = []
    for e in ([jnp.exp2(r - hi) for r in rows], [jnp.exp2(lo - r) for r in rows]):
        inv = _recip(_over_features(jnp.add, e))
        out += [t * inv for t in e]
    return jnp.concatenate(out, axis=0)


def _b_accumulate(i, x_ref, ln_ref, wb_ref, kv_ref, z_ref, phiq_ref):
    ln = ln_ref[_rows(i, TB), :]
    blocks = [slice(t * SUB, (t + 1) * SUB) for t in range(TB // SUB)]
    kv = {}

    def accumulate(ref, n, t):
        ref[n] = jnp.where(i > 0, ref[n], 0.0) + t

    for g in range(NG + 1):
        if g < NG:
            r = _nt(_unpack(wb_ref[g]), ln)
            for n in range(GP):
                pair = g * GP + n
                k, v, q = (r[j * GW + n * PF:j * GW + (n + 1) * PF] for j in range(3))
                phi_k, phi_q = _features(k), _pack(_features(q))
                kv[pair] = (v, phi_k.astype(bf16))
                accumulate(z_ref, pair, functools.reduce(jnp.add, [phi_k[:, b] for b in blocks]))
                for t, b in enumerate(blocks):
                    phiq_ref[i * len(blocks) + t, pair] = phi_q[:, b]
        for n in range((g - 1) * GP, g * GP) if g else ():
            accumulate(kv_ref, n, _nt(*kv.pop(n)))
    _store_ln(NSEG // UNROLL - 1, x_ref, ln_ref)


def _b_finish(kv_ref, z_ref):
    row, col = _iota((PF, 2 * PF), 0), _iota((PF, 2 * PF), 1)
    same_head = jnp.where(row >= F, 1, 0) == (col & 1)
    for n in range(NP):
        kv_ref[n] = jnp.where(same_head, kv_ref[n], 0.0)
        z_ref[n] = jnp.broadcast_to(jnp.sum(z_ref[n], axis=1, keepdims=True), (2 * PF, SUB))


def _b_output(i, out_copy, x_ref, io_ref, wob_ref, kv_ref, z_ref, phiq_ref):
    o = {}
    nsub = TB2 // SUB
    upper = _iota((8, SUB), 0) < F % 8
    for t in range(nsub + BLAG):
        if t < nsub:
            rows = []
            for n in range(NP):
                phi_q = _unpack(phiq_ref[i * nsub + t, n])
                num = _nn(kv_ref[n], phi_q)
                den = phi_q.astype(f32) * z_ref[n]
                den = _over_features(jnp.add, [den[r:r + 8] for r in range(0, 2 * PF, 8)])
                inv = 1.0 / (den + 1e-6)
                a, b = (jnp.broadcast_to(inv[j:j + 1], inv.shape) for j in range(2))
                rows += [num[8 * j:8 * j + 8] * c
                         for j, c in enumerate((a, a, jnp.where(upper, a, b), b, b))]
            o[t] = jnp.concatenate(rows, axis=0).astype(bf16)
        if t >= BLAG:
            blk = i * nsub + t - BLAG
            x = x_ref[_rows(blk, SUB), :] + _tn(o.pop(t - BLAG), _unpack(wob_ref[...]))
            x_ref[_rows(blk, SUB), :] = x
            io_ref[_rows(blk, SUB), :] = x.astype(bf16)
            out_copy(blk).start()


def _decode(row):
    pair = sum(jnp.where(row >= n * PF, 1, 0) for n in range(1, GP))
    return (row - pair * PF) >> 1, 2 * pair + (row & 1)


def _spread_phi(wphi_ref, phi_ref):
    hk, ck = _iota((H, D), 0), _iota((H, D), 1)
    phi = functools.reduce(
        jnp.add, [_nn(wphi_ref[d], _onehot(ck == hk * F + d)) for d in range(F)])
    spread = _onehot(_decode(_iota((GW, F), 0))[0] == _iota((GW, F), 1))
    phi_ref[...] = _nn(spread, phi.astype(bf16))


def _fold_phi(g, wqkv_ref, phi_ref, wb_ref):
    cw = 256

    def cols(base):
        return pl.ds(pl.multiple_of(base + g * 128, 128), cw)

    d = _iota((GW, cw), 1) - _decode(_iota((GW, cw), 0))[1] * F + g * (128 - GW)
    fold = jnp.where((d >= 0) & (d < F), phi_ref[:, cols(0)], 0.0).astype(bf16)
    wb_ref[g, 0:GW // 2] = _pack(_nt(fold, wqkv_ref[:, cols(D)]))
    wb_ref[g, GW:3 * GW // 2] = _pack(_nt(fold, wqkv_ref[:, cols(0)]))


def _kernel(x_hbm, x_tiles_hbm, mem0_hbm, wq_hbm, wk_hbm, wv_hbm, wo_hbm,
            bqkv_hbm, wphi_hbm, bwo_hbm, out_hbm,
            x_ref, h_ref, ln_ref, wqkv_ref, wo_ref, pre_ref, cap_ref,
            wb_ref, wob_ref, kv_ref, z_ref, phiq_ref,
            io_ref, lead_in_ref, lead_ref, stage_ref, bqkv_ref, bwo_ref, phi_ref,
            mem0_ref, wphi_ref, w_sem, sem, out_sem):
    first, rest = pl.ds(0, X_FIRST * SEG), pl.ds(X_FIRST * SEG, S - X_FIRST * SEG)
    x_first = pltpu.make_async_copy(x_hbm.at[first], io_ref.at[first], sem.at[0])
    x_rest = pltpu.make_async_copy(x_hbm.at[rest], io_ref.at[rest], sem.at[1])
    lead_copy = pltpu.make_async_copy(
        x_tiles_hbm.at[:, 0], lead_in_ref, sem.at[2])
    bqkv_copy = pltpu.make_async_copy(bqkv_hbm, bqkv_ref, sem.at[3])
    bwo_copy = pltpu.make_async_copy(bwo_hbm, bwo_ref, sem.at[4])
    mem0_copy = pltpu.make_async_copy(mem0_hbm, mem0_ref, sem.at[5])
    wphi_copy = pltpu.make_async_copy(wphi_hbm, wphi_ref, sem.at[6])

    def w_copy(p, j):
        src = (wq_hbm, wk_hbm, wv_hbm, wo_hbm)[j]
        return pltpu.make_async_copy(src.at[p], stage_ref.at[p, j], w_sem.at[p, j])

    def install(w, p, j):
        if j >= 2:
            w = jnp.concatenate(
                [w[r + c:r + c + 64] for c in range(0, DH, 64) for r in (0, DH)], axis=0)
        if j < 3:
            wqkv_ref[p, :, j * PW:(j + 1) * PW] = _pack(w.T)
        else:
            wo_ref[p] = _pack(w)

    early, late = (0, 1), (2, 3)
    wphi_copy.start()
    lead_copy.start()
    w_copy(0, 0).start()
    _store_caps(cap_ref)
    wphi_copy.wait()
    _spread_phi(wphi_ref, phi_ref)
    lead_copy.wait()
    w_copy(0, 1).start()
    for p in range(1, PREFETCH):
        for j in early:
            w_copy(p, j).start()
    lead_ref[...] = _layernorm(
        lead_in_ref[...].astype(f32).reshape(NSEG * V, D)).astype(bf16)

    def load_pair(p):
        for j in early:
            w_copy(p, j).wait()

        @pl.when(p >= LATE)
        def _():
            for j in late:
                w_copy(p - LATE, j).wait()

        @pl.when(p + PREFETCH < NP)
        def _():
            for j in early:
                w_copy(p + PREFETCH, j).start()

        @pl.when(p == LATE)
        def _():
            for copy in (bqkv_copy, bwo_copy, x_first, mem0_copy):
                copy.start()

        for j in late:
            w_copy(p, j).start()
        for j in early:
            install(stage_ref[p, j], p, j)
        due = p >= LATE
        for j in late:
            install(stage_ref[jnp.where(due, p - LATE, p), jnp.where(due, j, j - 2)],
                    jnp.where(due, p - LATE, p - LATE + NP), j)
        for j in early:
            for r in range(0, NSEG * V, 128):
                pre_ref[p, r:r + 128, j * PW:(j + 1) * PW] = _nt(
                    lead_ref[r:r + 128], stage_ref[p, j])

    pl.loop(0, NP)(load_pair)
    bqkv_copy.wait()
    bwo_copy.wait()

    @pl.loop(0, NG)
    def _(g):
        p = NP - LATE + g
        for j in late:
            w_copy(p, j).wait()
        _fold_phi(g, bqkv_ref, phi_ref, wb_ref)
        for j in late:
            install(stage_ref[p, j], p, j)

    wv = _pack(bqkv_ref[:, 2 * D:3 * D].T)
    for g in range(NG):
        wb_ref[g, GW // 2:GW] = wv[g * GW // 2:(g + 1) * GW // 2]
    wob_ref[...] = _pack(bwo_ref[...])
    x_first.wait()
    mem0_copy.wait()
    x_rest.start()
    x_ref[0:UNROLL * SEG, :] = io_ref[0:UNROLL * SEG, :].astype(f32)

    def out_copy(i):
        rows = _rows(i, SUB)
        return pltpu.make_async_copy(io_ref.at[rows], out_hbm.at[rows], out_sem)

    def wait_for_output():
        pltpu.make_async_copy(io_ref, out_hbm, out_sem).wait()

    def layer_a(layer):
        def read_x(s):
            return (x_ref if layer else io_ref)[_rows(s, SEG), :].astype(f32)

        h_ref[0:M, :] = mem0_ref[...].astype(f32)
        h_ref[M:L, :] = _layernorm(x_ref[0:SEG, :])

        @pl.loop(0, NSEG // UNROLL)
        def _(i):
            if layer == 0:
                pl.when(i == 1)(x_rest.wait)
            _a_steps(layer, i, read_x, x_ref, h_ref, ln_ref, wqkv_ref, wo_ref, pre_ref, cap_ref)

        if layer == 1:
            wait_for_output()

    @pl.loop(0, 2)
    def _(block):
        for layer in range(2):
            pl.when(block == layer)(functools.partial(layer_a, layer))
        pl.loop(0, S // TB)(
            lambda i: _b_accumulate(i, x_ref, ln_ref, wb_ref, kv_ref, z_ref, phiq_ref))
        _b_finish(kv_ref, z_ref)
        pl.loop(0, S // TB2)(
            lambda i: _b_output(i, out_copy, x_ref, io_ref, wob_ref, kv_ref, z_ref, phiq_ref))

    wait_for_output()


@functools.partial(jax.jit, static_argnames=("A_seg_len",))
def pallas_interleave_layers__memory_aug_recurrent_mem_tr__linear_kernel_hedgehog__prompt_kernel(
    A_x: jax.Array,
    A_mem0: jax.Array,
    A_Wq: jax.Array,
    A_Wk: jax.Array,
    A_Wv: jax.Array,
    A_Wo: jax.Array,
    A_seg_len: int,
    B_x: jax.Array,
    B_wqkv: jax.Array,
    B_w_phi: jax.Array,
    B_wo: jax.Array,
):
    del B_x
    assert A_x.shape == (1, S, D) and A_mem0.shape == (1, M, D) and A_seg_len == SEG
    assert A_Wq.shape == (D, H, DH) and B_w_phi.shape == (H, F, F)

    def head_major(w):
        return jnp.transpose(w, (1, 2, 0)).reshape(NP, PW, D)

    hbm = pl.BlockSpec(memory_space=pl.ANY)
    out = pl.pallas_call(
        _kernel,
        out_shape=jax.ShapeDtypeStruct((S, D), bf16),
        in_specs=[hbm] * 10,
        out_specs=hbm,
        scratch_shapes=[
            pltpu.VMEM((S, D), f32),
            pltpu.VMEM((L, D), f32),
            pltpu.VMEM((S, D), bf16),
            pltpu.VMEM((NP, D // 2, 3 * PW), u32),
            pltpu.VMEM((NP, PW // 2, D), u32),
            pltpu.VMEM((NP, NSEG * V, 2 * PW), f32),
            pltpu.VMEM((2 * L + 64, 128), f32),
            pltpu.VMEM((NG, 3 * GW // 2, D), u32),
            pltpu.VMEM((D // 2, D), u32),
            pltpu.VMEM((NP, PF, 2 * PF), f32),
            pltpu.VMEM((NP, 2 * PF, SUB), f32),
            pltpu.VMEM((S // SUB, NP, PF, SUB), u32),
            pltpu.VMEM((S, D), bf16),
            pltpu.VMEM((NSEG, V, D), bf16),
            pltpu.VMEM((NSEG * V, D), bf16),
            pltpu.VMEM((NP, 4, PW, D), bf16),
            pltpu.VMEM((D, 3 * D), bf16),
            pltpu.VMEM((D, D), bf16),
            pltpu.VMEM((GW, D), f32),
            pltpu.VMEM((M, D), bf16),
            pltpu.VMEM((F, F, H), bf16),
            pltpu.SemaphoreType.DMA((NP, 4)),
            pltpu.SemaphoreType.DMA((7,)),
            pltpu.SemaphoreType.DMA(()),
        ],
        compiler_params=pltpu.CompilerParams(vmem_limit_bytes=120 * 1024 * 1024),
    )(
        A_x.reshape(S, D),
        A_x.reshape(NSEG, SEG // V, V, D),
        A_mem0.reshape(M, D),
        head_major(A_Wq),
        head_major(A_Wk),
        head_major(A_Wv),
        A_Wo.reshape(NP, PW, D),
        B_wqkv,
        jnp.transpose(B_w_phi, (1, 2, 0)),
        B_wo,
    )
    return out.reshape(1, S, D)
```
